```python
import jax
import jax.numpy as jnp

def _softmax(x, axis=-1):
    return jax.nn.softmax(x, axis=axis)
def _gelu(x):
    return jax.nn.gelu(x, approximate=True)
def _silu(x):
    return jax.nn.silu(x)
def _sigmoid(x):
    return jax.nn.sigmoid(x)
def _layernorm(x, axis=-1, eps=1e-5):
    m = jnp.mean(x, axis=axis, keepdims=True)
    v = jnp.var(x, axis=axis, keepdims=True)
    return (x - m) / jnp.sqrt(v + eps)
def _scatter_add(tgt, idx, src, axis=0):
    return tgt.at[idx].add(src)
def _segment_sum(src, seg, n):
    return jax.ops.segment_sum(src, seg, n)
class _Rng:
    def __init__(self, key):
        self._k = key
    def _next(self):
        self._k, sub = jax.random.split(self._k)
        return sub
    def normal(self, shape):
        return jax.random.normal(self._next(), shape, dtype=jnp.bfloat16)
    def randint(self, lo, hi, shape):
        return jax.random.randint(self._next(), shape, lo, hi, dtype=jnp.int32)
    def uniform(self, shape, lo=0.0, hi=1.0):
        return jax.random.uniform(self._next(), shape, jnp.bfloat16, lo, hi)
    def permutation(self, n):
        return jax.random.permutation(self._next(), n)


kernel_name = 'interleave_layers__sliding_block_cached__glu_gated_swiglu__decode'

def setup_inputs():
    _rng = _Rng(jax.random.key(int.from_bytes(__import__("os").urandom(4), "little")))
    _w = (lambda a: (lambda t: t.astype(jnp.bfloat16) if jnp.issubdtype(t.dtype, jnp.floating) else t)(jnp.asarray(a)))
    def _A_setup():
        B, Sq, D = 1, 1, 640
        Hq, Hkv, Sk, Dh = 32, 32, 32768, 192
        assert Hq % Hkv == 0, (Hq, Hkv)
        return {
            "x": _w((lambda *s: _rng.normal(s) * 0.05)(B, Sq, D)),
            "k_cache": _w((lambda *s: _rng.normal(s) * 0.05)(B, Hkv, Sk, Dh)),
            "v_cache": _w((lambda *s: _rng.normal(s) * 0.05)(B, Hkv, Sk, Dh)),
            "wq": _w((lambda *s: _rng.normal(s) * 0.05)(D, Hq * Dh) * (D ** -0.5)),
            "wo": _w((lambda *s: _rng.normal(s) * 0.05)(Hq * Dh, D) * ((Hq * Dh) ** -0.5)),
        }
    _A_in = _A_setup()

    def _B_setup():
        B, S, D, F = 1, 1, 640, 1536
        return {
            "x": _w((lambda *s: _rng.normal(s) * 0.05)(B, S, D)),
            "w1": _w((lambda *s: _rng.normal(s) * 0.05)(D, F) * (2.0 / D) ** 0.5),
            "w3": _w((lambda *s: _rng.normal(s) * 0.05)(D, F) * (2.0 / D) ** 0.5),
            "w2": _w((lambda *s: _rng.normal(s) * 0.05)(F, D) * (2.0 / F) ** 0.5),
        }
    _B_in = _B_setup()

    return {
        "A_x": _A_in["x"],
        "A_k_cache": _A_in["k_cache"],
        "A_v_cache": _A_in["v_cache"],
        "A_wq": _A_in["wq"],
        "A_wo": _A_in["wo"],
        "B_x": _B_in["x"],
        "B_w1": _B_in["w1"],
        "B_w3": _B_in["w3"],
        "B_w2": _B_in["w2"],
    }

def reference(A_x, A_k_cache, A_v_cache, A_wq, A_wo, B_x, B_w1, B_w3, B_w2):
    def _A_ref(x, k_cache, v_cache, wq, wo):
        B, Sq, D = x.shape
        Hq, Dh = 32, 192
        Hkv, Sk = k_cache.shape[1], k_cache.shape[2]
        W = min(4096, max(256, Sk // 4))
        rep = Hq // Hkv
        q = (lambda x, *d: x.transpose(*d))((x @ wq).reshape(B, Sq, Hq, Dh), 0, 2, 1, 3)
        k = jnp.repeat(k_cache[:, :, Sk - W:, :], rep, axis=1)
        v = jnp.repeat(v_cache[:, :, Sk - W:, :], rep, axis=1)
        scores = jnp.einsum("bhqd,bhkd->bhqk", q, k) * (Dh ** -0.5)
        p = _softmax(scores, axis=-1)
        o = jnp.einsum("bhqk,bhkd->bhqd", p, v)
        return (lambda x, *d: x.transpose(*d))(o, 0, 2, 1, 3).reshape(B, Sq, Hq * Dh) @ wo

    def _B_ref(x, w1, w3, w2):
        gate = jnp.einsum("bsd,df->bsf", x, w1)
        up = jnp.einsum("bsd,df->bsf", x, w3)
        h = _silu(gate) * up
        out = jnp.einsum("bsf,fd->bsd", h, w2)
        return out

    x = A_x
    x = x + _A_ref(_layernorm(x, axis=-1), A_k_cache, A_v_cache, A_wq, A_wo)
    x = x + _B_ref(_layernorm(x, axis=-1), B_w1, B_w3, B_w2)
    x = x + _A_ref(_layernorm(x, axis=-1), A_k_cache, A_v_cache, A_wq, A_wo)
    x = x + _B_ref(_layernorm(x, axis=-1), B_w1, B_w3, B_w2)
    return x
```

```python
import jax
import jax.numpy as jnp
from jax import lax
import jax.experimental.pallas as pl
import jax.experimental.pallas.tpu as pltpu

F32, BF16, U32 = jnp.float32, jnp.bfloat16, jnp.uint32

D, HQ, DH, FF = 640, 32, 192, 1536
NP = HQ // 2
PR = 2 * DH
KC, NC, FC = D // 128, PR // 128, FF // 128
EPS = 1e-5
SCALE = DH ** -0.5

MXU_TILES_STEADY = 2
MXU_TILES_LAST = 16
W2_CHUNKS = 4


def _bf(w):
    return pltpu.bitcast(w, BF16)


def _mm(lhs, w):
    return lax.dot_general(lhs, _bf(w), (((1,), (0,)), ((), ())),
                           preferred_element_type=F32)


def _mm_t(lhs, w):
    return lax.dot_general(lhs, _bf(w), (((1,), (1,)), ((), ())),
                           preferred_element_type=F32)


def _round(x):
    return x.astype(BF16).astype(F32)


def _tree_sum(xs):
    xs = list(xs)
    while len(xs) > 1:
        xs = [xs[i] + xs[i + 1] if i + 1 < len(xs) else xs[i]
              for i in range(0, len(xs), 2)]
    return xs[0]


def _layernorm(x):
    m = jnp.mean(x, axis=-1, keepdims=True)
    c = x - m
    v = jnp.mean(c * c, axis=-1, keepdims=True)
    return _round(c * lax.rsqrt(v + EPS))


def _interleave(a, na, b, nb):
    ia = ib = 0
    while ia < na or ib < nb:
        if ib >= nb or (ia < na and ia * nb <= ib * na):
            next(a, None)
            ia += 1
        else:
            next(b, None)
            ib += 1
    for _ in a:
        pass
    for _ in b:
        pass


def _make_kernel(s0, win):
    nt = win // 128
    nu = nt // 4

    def kernel(x_hbm, k_hbm, v_hbm, wq_hbm, wo_hbm, w1_hbm, w3_hbm, w2_hbm, o_ref,
               kb, vb, wqb, wob, w1b, w3b, w2b, xb,
               xn_s, qp, sa, sb, pb, lp, ab, ox, yp, yacc,
               sem_k, sem_v, sem_q, sem_w):
        row = lax.broadcasted_iota(jnp.int32, (8, 128), 0)
        lane = lax.broadcasted_iota(jnp.int32, (8, 128), 1)

        def kv_copy(src, dst, sem, g):
            return pltpu.make_async_copy(
                src.at[g, :, pl.ds(s0, win)], dst.bitcast(BF16).at[g], sem.at[g])

        def k_copy(g):
            return kv_copy(k_hbm, kb, sem_k, g)

        def v_copy(g):
            return kv_copy(v_hbm, vb, sem_v, g)

        def wq_copy(g):
            return pltpu.make_async_copy(
                wq_hbm.at[:, pl.ds(g * PR, PR)], wqb.bitcast(BF16).at[g], sem_q.at[g])

        x_copy = pltpu.make_async_copy(x_hbm, xb, sem_w.at[0])
        wo_copy = pltpu.make_async_copy(wo_hbm, wob.bitcast(BF16), sem_w.at[1])
        w1_copy = pltpu.make_async_copy(w1_hbm, w1b.bitcast(BF16), sem_w.at[2])
        w3_copy = pltpu.make_async_copy(w3_hbm, w3b.bitcast(BF16), sem_w.at[3])
        w2_rows = FF // W2_CHUNKS

        def w2_copy(c):
            return pltpu.make_async_copy(
                w2_hbm.at[pl.ds(c * w2_rows, w2_rows)],
                w2b.bitcast(BF16).at[pl.ds(c * w2_rows, w2_rows)], sem_w.at[4 + c])

        k_copy(0).start()
        x_copy.start()
        for g in range(NP):
            wq_copy(g).start()
        wo_copy.start()
        k_copy(1).start()
        v_copy(0).start()

        def mxu_q(g):
            for n in range(NC):
                for c in range(KC):
                    qp[c, :, n * 128:(n + 1) * 128] = _mm(
                        xn_s[:, c * 128:(c + 1) * 128],
                        wqb[g, c * 64:(c + 1) * 64, n * 128:(n + 1) * 128])
                    yield

        def q_lhs():
            q = _round(_tree_sum(qp[c] for c in range(KC)))
            mid = jnp.where((row & 1) == (lane >> 6), q[:, 128:256], 0.0)
            return q[:, :128], mid, q[:, 256:]

        def mxu_scores(g, lhs):
            for t in range(nt):
                u, r = t // 4, 2 * (t % 4)
                cols = slice(t * 128, (t + 1) * 128)
                sa[u, r:r + 1, :] = _mm(lhs[0], kb[g, 0:64, cols])[r:r + 1]
                yield
                sb[u, r:r + 2, :] = _mm(lhs[1], kb[g, 64:128, cols])[r:r + 2]
                yield
                sa[u, r + 1:r + 2, :] = _mm(lhs[2], kb[g, 128:192, cols])[r + 1:r + 2]
                yield

        def mxu_pv(g, tiles):
            for t in tiles:
                u, r = t // 4, 2 * (t % 4)
                p = pb[u]
                for j in range(NC):
                    ox[u, r:r + 2, j * 128:(j + 1) * 128] = _mm_t(
                        p, vb[g, j * 64:(j + 1) * 64, t * 128:(t + 1) * 128])[r:r + 2]
                    yield

        def mxu_wo(g, o):
            for j in range(NC):
                for n in range(KC):
                    yp[j, :, n * 128:(n + 1) * 128] = _mm(
                        o[j], wob[g, j * 64:(j + 1) * 64, n * 128:(n + 1) * 128])
                    yield

        def vpu_pv(g, tiles):
            for h in range(2):
                acc = [None] * (DH // 16)
                for t in tiles:
                    r = 2 * (t % 4) + h
                    p = jnp.broadcast_to(pb[t // 4, r:r + 1, :], (16, 128))
                    for i in range(DH // 16):
                        r0 = h * (DH // 2) + i * 8
                        v = _bf(vb[g, r0:r0 + 8, t * 128:(t + 1) * 128]).astype(F32) * p
                        acc[i] = v if acc[i] is None else acc[i] + v
                        yield
                for i in range(DH // 16):
                    ab[h * DH + i * 16:h * DH + (i + 1) * 16, :] = acc[i]

        def per_head(x, op):
            x = op(x, pltpu.roll(x, 2, 0))
            return op(x, pltpu.roll(x, 4, 0))

        def softmax(g):
            s = [sa[u] + sb[u] for u in range(nu)]
            m = s[0]
            for x in s[1:]:
                m = jnp.maximum(m, x)
            m = jnp.max(per_head(m, jnp.maximum), axis=1, keepdims=True)
            p = [jnp.exp((x - m) * SCALE) for x in s]
            for u in range(nu):
                pb[u] = p[u]
            lp[g] = _tree_sum(p)

        def pv_finish(g, mxu_tiles):
            l = jnp.sum(per_head(lp[g], jnp.add), axis=1, keepdims=True)
            inv = jnp.broadcast_to(1.0 / l, (8, 128))
            inv_o = pltpu.roll(inv, 1, 0)
            even = (row & 1) == 0
            inv_a, inv_b = jnp.where(even, inv, inv_o), jnp.where(even, inv_o, inv)
            scale = (inv_a, jnp.where(lane < 64, inv_a, inv_b), inv_b)
            own = (even, (row & 1) == (lane >> 6), jnp.logical_not(even))
            out = []
            for j in range(NC):
                part = []
                if len(mxu_tiles) < nt:
                    at = ab[j * 128:(j + 1) * 128, :].T
                    part = [at[i * 8:(i + 1) * 8] for i in range(16)]
                for u in sorted({t // 4 for t in mxu_tiles}):
                    n_rows = 2 * sum(t // 4 == u for t in mxu_tiles)
                    keep = own[j] if n_rows == 8 else jnp.logical_and(own[j], row < n_rows)
                    part.append(jnp.where(keep, ox[u, :, j * 128:(j + 1) * 128], 0.0))
                o = _tree_sum(part)
                o = o + pltpu.roll(o, 1, 0)
                out.append(_round(per_head(o, jnp.add) * scale[j]))
            return out

        def add_y():
            yacc[...] += _tree_sum(yp[j] for j in range(NC))

        steady = list(range(nt - nt // 8 * 4, nt))[:MXU_TILES_STEADY]
        last = list(range(nt - min(MXU_TILES_LAST, nt), nt))

        def stage(g, *, q_next, scores, pv, wo, y):
            if y:
                add_y()
            mxu, n_mxu, vpu, n_vpu = [], 0, iter(()), 0
            if scores:
                mxu.append(mxu_scores(g, q_lhs()))
                n_mxu += NC * nt
            if wo is not None:
                o = pv_finish(g - 2, wo)
            if pv is not None:
                mxu.append(mxu_pv(g - 1, pv))
                n_mxu += NC * len(pv)
                tiles = [t for t in range(nt) if t not in pv]
                vpu, n_vpu = vpu_pv(g - 1, tiles), len(tiles) * PR // 16
            if q_next:
                mxu.append(mxu_q(g + 1))
                n_mxu += NC * KC
            if wo is not None:
                mxu.append(mxu_wo(g - 2, o))
                n_mxu += NC * KC
            _interleave((None for s in mxu for _ in s), n_mxu, vpu, n_vpu)
            if scores:
                softmax(g)

        def layer(it, x):
            first = it == 0

            def when_first(*copies, start=()):
                @pl.when(first)
                def _():
                    for c in start:
                        c().start()
                    for c in copies:
                        c().wait()

            xn_s[...] = _layernorm(x)
            yacc[...] = jnp.zeros_like(yacc)
            when_first(*[lambda g=g: wq_copy(g) for g in range(NP)], lambda: k_copy(0))
            for _ in mxu_q(0):
                pass
            stage(0, q_next=True, scores=True, pv=None, wo=None, y=False)
            when_first(lambda: wo_copy, lambda: k_copy(1), lambda: v_copy(0),
                       start=(lambda: k_copy(2), lambda: v_copy(1)))
            stage(1, q_next=True, scores=True, pv=steady, wo=None, y=False)
            yp[...] = jnp.zeros_like(yp)

            def body(g, carry):
                when_first(lambda: k_copy(g), lambda: v_copy(g - 1),
                           start=(lambda: k_copy(g + 1), lambda: v_copy(g)))
                stage(g, q_next=True, scores=True, pv=steady, wo=steady, y=True)
                return carry

            lax.fori_loop(2, NP - 1, body, 0)
            when_first(lambda: k_copy(NP - 1), lambda: v_copy(NP - 2),
                       start=(lambda: v_copy(NP - 1),))
            stage(NP - 1, q_next=False, scores=True, pv=steady, wo=steady, y=True)
            when_first(lambda: v_copy(NP - 1),
                       start=(lambda: w1_copy, lambda: w3_copy,
                              *[lambda c=c: w2_copy(c) for c in range(W2_CHUNKS)]))
            stage(NP, q_next=False, scores=False, pv=last, wo=steady, y=True)
            stage(NP + 1, q_next=False, scores=False, pv=None, wo=last, y=True)
            x = _round(x + _round(yacc[...] + _tree_sum(yp[j] for j in range(NC))))

            xn = _layernorm(x)
            when_first(lambda: w1_copy, lambda: w3_copy)
            h = []
            for f in range(FC):
                cols = slice(f * 128, (f + 1) * 128)
                gate, up = (
                    _round(_tree_sum(
                        _mm(xn[:, c * 128:(c + 1) * 128], w[c * 64:(c + 1) * 64, cols])
                        for c in range(KC)))
                    for w in (w1b, w3b))
                h.append(_round(_round(gate * jax.nn.sigmoid(gate)) * up))
            y = [None] * KC
            per = FC // W2_CHUNKS
            for c in range(W2_CHUNKS):
                when_first(lambda c=c: w2_copy(c))
                for f in range(c * per, (c + 1) * per):
                    for n in range(KC):
                        r = _mm(h[f], w2b[f * 64:(f + 1) * 64, n * 128:(n + 1) * 128])
                        y[n] = r if y[n] is None else y[n] + r
            return _round(x + _round(jnp.concatenate(y, axis=1)))

        x_copy.wait()
        x = jnp.broadcast_to(xb[0].astype(F32), (8, D))
        x = lax.fori_loop(0, 2, layer, x)
        o_ref[0] = x[0:1].astype(o_ref.dtype)

    return kernel, nu


@jax.jit
def pallas_interleave_layers__sliding_block_cached__glu_gated_swiglu__decode_kernel(
    A_x: jax.Array,
    A_k_cache: jax.Array,
    A_v_cache: jax.Array,
    A_wq: jax.Array,
    A_wo: jax.Array,
    B_x: jax.Array,
    B_w1: jax.Array,
    B_w3: jax.Array,
    B_w2: jax.Array,
):
    del B_x
    sk = A_k_cache.shape[2]
    win = min(4096, max(256, sk // 4))
    assert A_x.shape == (1, 1, D) and A_k_cache.shape == (1, HQ, sk, DH)
    assert win % 1024 == 0 and (sk - win) % 128 == 0
    kernel, nu = _make_kernel(sk - win, win)

    def as_rows(c):
        return jnp.swapaxes(c, 2, 3).reshape(NP, PR, sk)

    return pl.pallas_call(
        kernel,
        out_shape=jax.ShapeDtypeStruct((1, 1, D), A_x.dtype),
        in_specs=[pl.BlockSpec(memory_space=pl.ANY)] * 8,
        scratch_shapes=[
            pltpu.VMEM((NP, PR // 2, win), U32),
            pltpu.VMEM((NP, PR // 2, win), U32),
            pltpu.VMEM((NP, D // 2, PR), U32),
            pltpu.VMEM((NP, PR // 2, D), U32),
            pltpu.VMEM((D // 2, FF), U32),
            pltpu.VMEM((D // 2, FF), U32),
            pltpu.VMEM((FF // 2, D), U32),
            pltpu.VMEM((1, 1, D), BF16),
            pltpu.VMEM((8, D), F32),
            pltpu.VMEM((KC, 8, PR), F32),
            pltpu.VMEM((nu, 8, 128), F32),
            pltpu.VMEM((nu, 8, 128), F32),
            pltpu.VMEM((nu, 8, 128), F32),
            pltpu.VMEM((NP, 8, 128), F32),
            pltpu.VMEM((PR, 128), F32),
            pltpu.VMEM((nu, 8, PR), F32),
            pltpu.VMEM((NC, 8, D), F32),
            pltpu.VMEM((8, D), F32),
            pltpu.SemaphoreType.DMA((NP,)),
            pltpu.SemaphoreType.DMA((NP,)),
            pltpu.SemaphoreType.DMA((NP,)),
            pltpu.SemaphoreType.DMA((4 + W2_CHUNKS,)),
        ],
        compiler_params=pltpu.CompilerParams(vmem_limit_bytes=126 * 1024 * 1024),
        name="interleave_decode",
    )(A_x, as_rows(A_k_cache), as_rows(A_v_cache), A_wq, A_wo.reshape(NP, PR, D),
      B_w1, B_w3, B_w2)
```

```python
import jax
import jax.numpy as jnp
from jax import lax
import jax.experimental.pallas as pl
import jax.experimental.pallas.tpu as pltpu

F32, BF16, U32 = jnp.float32, jnp.bfloat16, jnp.uint32

D, HQ, DH, FF = 640, 32, 192, 1536
NP = HQ // 2
PR = 2 * DH
KC, NC, FC = D // 128, PR // 128, FF // 128
EPS = 1e-5
SCALE = DH ** -0.5

MXU_TILES_STEADY = 2
MXU_TILES_LAST = 16
W2_CHUNKS = 4
PV_BLOCK = 3
MXU_LEAD = 4


def _bf(w):
    return pltpu.bitcast(w, BF16)


def _mm(lhs, w):
    return lax.dot_general(lhs, _bf(w), (((1,), (0,)), ((), ())),
                           preferred_element_type=F32)


def _mm_t(lhs, w):
    return lax.dot_general(lhs, _bf(w), (((1,), (1,)), ((), ())),
                           preferred_element_type=F32)


def _round(x):
    return x.astype(BF16).astype(F32)


def _tree_sum(xs):
    xs = list(xs)
    while len(xs) > 1:
        xs = [xs[i] + xs[i + 1] if i + 1 < len(xs) else xs[i]
              for i in range(0, len(xs), 2)]
    return xs[0]


def _layernorm(x):
    m = jnp.mean(x, axis=-1, keepdims=True)
    c = x - m
    v = jnp.mean(c * c, axis=-1, keepdims=True)
    return _round(c * lax.rsqrt(v + EPS))


def _interleave(a, na, lead, b, nb):
    ia = ib = 0
    while ia < na or ib < nb:
        if ib >= nb or (ia < na and (ia - lead) * nb <= ib * na):
            ia += next(a)
        else:
            ib += next(b)
    for _ in a:
        pass
    for _ in b:
        pass


def _make_kernel(s0, win):
    nt = win // 128
    nu = nt // 4

    def kernel(x_hbm, k_hbm, v_hbm, wq_hbm, wo_hbm, w1_hbm, w3_hbm, w2_hbm, o_ref,
               kb, vb, wqb, wob, w1b, w3b, w2b, xb,
               xn_s, qp, ql, sa, sb, pb, pbb, lp, ox, yp, yacc,
               sem_k, sem_v, sem_w):
        row = lax.broadcasted_iota(jnp.int32, (8, 128), 0)
        lane = lax.broadcasted_iota(jnp.int32, (8, 128), 1)

        class Copy:
            def __init__(self, src, col0, buf, idx, n, sem):
                self.src, self.col0, self.buf, self.idx = src, col0, buf, idx
                self.n, self.sem = n, sem

            def start(self):
                def one(i, carry):
                    col = pl.multiple_of(self.col0 + i * 128, 128)
                    src = self.src.at[(slice(None),) * (len(self.src.shape) - 1)
                                      + (pl.ds(col, 128),)]
                    dst = self.buf.bitcast(BF16).at[self.idx(i, 2)]
                    pltpu.make_async_copy(src, dst, self.sem).start()
                    return carry
                lax.fori_loop(0, self.n, one, 0)

            def wait(self):
                whole = self.buf.at[self.idx(pl.ds(0, self.n), 1)]
                pltpu.make_async_copy(whole, whole, self.sem).wait()

        def k_copy(g):
            return Copy(k_hbm.at[g], s0, kb, lambda i, _: (g, i), nt, sem_k.at[g])

        def v_copy(g):
            return Copy(v_hbm.at[g], s0, vb, lambda i, _: (g, i), nt, sem_v.at[g])

        x_copy = pltpu.make_async_copy(x_hbm, xb, sem_w.at[0])
        wq_copy = Copy(wq_hbm, 0, wqb, lambda i, _: (i,), NP * NC, sem_w.at[1])
        wo_copy = Copy(wo_hbm, 0, wob, lambda i, _: (i, pl.ds(0, NP)), KC, sem_w.at[2])
        w1_copy = Copy(w1_hbm, 0, w1b, lambda i, _: (i,), FC, sem_w.at[3])
        w3_copy = Copy(w3_hbm, 0, w3b, lambda i, _: (i,), FC, sem_w.at[4])
        w2_rows = FF // W2_CHUNKS // 2

        def w2_copy(c):
            return Copy(w2_hbm.at[pl.ds(2 * c * w2_rows, 2 * w2_rows)], 0, w2b,
                        lambda i, m: (i, pl.ds(m * c * w2_rows, m * w2_rows)),
                        KC, sem_w.at[5 + c])

        x_copy.start()
        wq_copy.start()
        k_copy(0).start()

        newest = []

        def fence(ref):
            if newest:
                ref[0:8, :] = newest[0][0:8]

        def mxu_q(g):
            fence(wqb.at[NP * NC])
            for n in range(NC):
                for c in range(KC):
                    qp[c, :, n * 128:(n + 1) * 128] = _mm(
                        xn_s[:, c * 128:(c + 1) * 128],
                        wqb[g * NC + n, c * 64:(c + 1) * 64, :])
                    yield 1

        def q_finish():
            q = _round(_tree_sum(qp[c] for c in range(KC)))
            ql[0] = q[:, :128]
            ql[1] = jnp.where((row & 1) == (lane >> 6), q[:, 128:256], 0.0)
            ql[2] = q[:, 256:]

        def mxu_scores(g):
            lhs = [ql[j] for j in range(NC)]
            for t in range(nt):
                u, r = t // 4, 2 * (t % 4)
                sa[u, r:r + 1, :] = _mm(lhs[0], kb[g, t, 0:64, :])[r:r + 1]
                yield 1
                sb[u, r:r + 2, :] = _mm(lhs[1], kb[g, t, 64:128, :])[r:r + 2]
                yield 1
                sa[u, r + 1:r + 2, :] = _mm(lhs[2], kb[g, t, 128:192, :])[r + 1:r + 2]
                yield 1

        def mxu_pv(g, tiles):
            for t in tiles:
                u, r = t // 4, 2 * (t % 4)
                p = pb[u]
                for j in range(NC):
                    ox[u, r:r + 2, j * 128:(j + 1) * 128] = _mm_t(
                        p, vb[g, t, j * 64:(j + 1) * 64, :])[r:r + 2]
                    yield 2

        def mxu_wo(g, spare):
            fence(wob.at[0, NP])
            for j in range(NC):
                o = pltpu.bitcast(kb[spare, j, 128:136, :], F32)
                for n in range(KC):
                    yp[j, :, n * 128:(n + 1) * 128] = _mm(
                        o, wob[n, g, j * 64:(j + 1) * 64, :])
                    yield 1

        def vpu_pv(g, tiles, filler):
            for h in range(2):
                for i0 in range(0, DH // 16, PV_BLOCK):
                    acc = [None] * PV_BLOCK
                    for t in tiles:
                        if i0 == 0:
                            r = 2 * (t % 4) + h
                            p = jnp.broadcast_to(pb[t // 4, r:r + 1, :], (8, 128))
                            pbb[h, t] = p
                        else:
                            p = pbb[h, t]
                        p = jnp.concatenate([p, p], axis=0)
                        for i in range(PV_BLOCK):
                            r0 = h * (DH // 2) + (i0 + i) * 8
                            v = _bf(vb[g, t, r0:r0 + 8, :]).astype(F32) * p
                            acc[i] = v if acc[i] is None else acc[i] + v
                        if t == tiles[-1]:
                            for i in range(PV_BLOCK):
                                j, r0 = divmod(h * DH + (i0 + i) * 16, 128)
                                newest[:] = [pltpu.bitcast(acc[i], U32)]
                                kb[NP, j, r0:r0 + 16, :] = newest[0]
                        if t in (tiles[len(tiles) // 4], tiles[3 * len(tiles) // 4]):
                            next(filler, None)
                        yield PV_BLOCK

        def per_head(x, op):
            x = op(x, pltpu.roll(x, 2, 0))
            return op(x, pltpu.roll(x, 4, 0))

        def softmax(g):
            s = [sa[u] + sb[u] for u in range(nu)]
            m = s[0]
            for x in s[1:]:
                m = jnp.maximum(m, x)
            m = jnp.max(per_head(m, jnp.maximum), axis=1, keepdims=True)
            p = [jnp.exp((x - m) * SCALE) for x in s]
            for u in range(nu):
                pb[u] = p[u]
            lp[g] = _tree_sum(p)

        def pv_finish(g, mxu_tiles, spare):
            l = jnp.sum(per_head(lp[g], jnp.add), axis=1, keepdims=True)
            inv = jnp.broadcast_to(1.0 / l, (8, 128))
            inv_o = pltpu.roll(inv, 1, 0)
            even = (row & 1) == 0
            inv_a, inv_b = jnp.where(even, inv, inv_o), jnp.where(even, inv_o, inv)
            scale = (inv_a, jnp.where(lane < 64, inv_a, inv_b), inv_b)
            own = (even, (row & 1) == (lane >> 6), jnp.logical_not(even))
            extra = [[] for _ in range(NC)]
            for u in sorted({t // 4 for t in mxu_tiles}):
                n_rows = 2 * sum(t // 4 == u for t in mxu_tiles)
                for j in range(NC):
                    keep = own[j] if n_rows == 8 else jnp.logical_and(own[j], row < n_rows)
                    extra[j].append(jnp.where(keep, ox[u, :, j * 128:(j + 1) * 128], 0.0))
            for j in range(NC):
                if len(mxu_tiles) < nt:
                    diag = jnp.zeros((8, 128), F32)
                    for i in range(16):
                        acc = pltpu.bitcast(kb[spare, j, i * 8:(i + 1) * 8, :], F32)
                        diag = jnp.where(lane - row == 8 * i,
                                         jnp.sum(acc, axis=1, keepdims=True), diag)
                        if i == 7:
                            yield
                            kb[NP, j, 128:136, :] = pltpu.bitcast(diag, U32)
                    yield
                    extra[j].append(diag)
                o = _tree_sum(extra[j])
                o = o + pltpu.roll(o, 1, 0)
                o = _round(per_head(o, jnp.add) * scale[j])
                kb[NP, j, 128:136, :] = pltpu.bitcast(o, U32)

        def add_y():
            yacc[...] += _tree_sum(yp[j] for j in range(NC))

        steady = list(range(nt - nt // 8 * 4, nt))[:MXU_TILES_STEADY]
        last = list(range(nt - min(MXU_TILES_LAST, nt), nt))

        def stage(g, spare, *, q_next, scores, pv, wo, y):
            if y:
                add_y()
            mxu, n_mxu, vpu, n_vpu, filler = [], 0, iter(()), 0, iter(())
            newest.clear()
            if wo is not None:
                filler = pv_finish(g - 2, wo, spare)
                next(filler, None)
            tiles = [] if pv is None else [t for t in range(nt) if t not in pv]
            if tiles:
                vpu, n_vpu = vpu_pv(g - 1, tiles, filler), len(tiles) * PR // 16
            else:
                for _ in filler:
                    pass
            if pv is not None:
                mxu.append(mxu_pv(g - 1, pv))
                n_mxu += 2 * NC * len(pv)
            if scores:
                mxu.append(mxu_scores(g))
                n_mxu += NC * nt
            if q_next:
                mxu.append(mxu_q(g + 1))
                n_mxu += NC * KC
            if wo is not None:
                mxu.append(mxu_wo(g - 2, spare))
                n_mxu += NC * KC
            _interleave((w for s in mxu for w in s), n_mxu, MXU_LEAD, vpu, n_vpu)
            if scores:
                softmax(g)
            if q_next:
                q_finish()

        def layer(it, x):
            first = it == 0
            z = it >> 1

            def when_first(*copies, start=()):
                @pl.when(first)
                def _():
                    for c in start:
                        c().start()
                    for c in copies:
                        c().wait()

            xn_s[...] = _layernorm(x)
            yacc[...] = jnp.zeros_like(yacc)
            when_first(lambda: wq_copy, lambda: k_copy(0),
                       start=(lambda: wo_copy, lambda: k_copy(1), lambda: v_copy(0)))
            newest.clear()
            for _ in mxu_q(0):
                pass
            q_finish()
            stage(z, NP + z, q_next=True, scores=True, pv=None, wo=None, y=False)
            when_first(lambda: wo_copy, lambda: k_copy(1), lambda: v_copy(0),
                       start=(lambda: k_copy(2), lambda: v_copy(1)))
            stage(1 + z, NP + z, q_next=True, scores=True, pv=steady, wo=None, y=False)
            yp[...] = jnp.zeros_like(yp)

            def body(g, carry):
                when_first(lambda: k_copy(g), lambda: v_copy(g - 1),
                           start=(lambda: k_copy(g + 1), lambda: v_copy(g)))
                stage(g, NP + z, q_next=True, scores=True, pv=steady, wo=steady, y=True)
                return carry

            lax.fori_loop(2, NP - 1, body, 0)
            when_first(lambda: k_copy(NP - 1), lambda: v_copy(NP - 2),
                       start=(lambda: v_copy(NP - 1),))
            stage(NP - 1 + z, NP + z, q_next=False, scores=True, pv=steady, wo=steady, y=True)
            when_first(lambda: v_copy(NP - 1),
                       start=(lambda: w1_copy, lambda: w3_copy,
                              *[lambda c=c: w2_copy(c) for c in range(W2_CHUNKS)]))
            stage(NP + z, NP + z, q_next=False, scores=False, pv=last, wo=steady, y=True)
            stage(NP + 1, NP, q_next=False, scores=False, pv=None, wo=last, y=True)
            x = _round(x + _round(yacc[...] + _tree_sum(yp[j] for j in range(NC))))

            xn = _layernorm(x)
            when_first(lambda: w1_copy, lambda: w3_copy)
            h = []
            for f in range(FC):
                gate, up = (
                    _round(_tree_sum(
                        _mm(xn[:, c * 128:(c + 1) * 128], w[f, c * 64:(c + 1) * 64, :])
                        for c in range(KC)))
                    for w in (w1b, w3b))
                h.append(_round(_round(gate * jax.nn.sigmoid(gate)) * up))
            y = [None] * KC
            per = FC // W2_CHUNKS
            for c in range(W2_CHUNKS):
                when_first(lambda c=c: w2_copy(c))
                for f in range(c * per, (c + 1) * per):
                    for n in range(KC):
                        r = _mm(h[f], w2b[n, f * 64:(f + 1) * 64, :])
                        y[n] = r if y[n] is None else y[n] + r
            return _round(x + _round(jnp.concatenate(y, axis=1)))

        x_copy.wait()
        x = jnp.broadcast_to(xb[0].astype(F32), (8, D))
        x = lax.fori_loop(0, 2, layer, x)
        o_ref[0] = x[0:1].astype(o_ref.dtype)

    return kernel, nu


@jax.jit
def pallas_interleave_layers__sliding_block_cached__glu_gated_swiglu__decode_kernel(
    A_x: jax.Array,
    A_k_cache: jax.Array,
    A_v_cache: jax.Array,
    A_wq: jax.Array,
    A_wo: jax.Array,
    B_x: jax.Array,
    B_w1: jax.Array,
    B_w3: jax.Array,
    B_w2: jax.Array,
):
    del B_x
    sk = A_k_cache.shape[2]
    win = min(4096, max(256, sk // 4))
    assert A_x.shape == (1, 1, D) and A_k_cache.shape == (1, HQ, sk, DH)
    assert win % 1024 == 0 and (sk - win) % 128 == 0
    kernel, nu = _make_kernel(sk - win, win)

    def as_rows(c):
        return jnp.swapaxes(c, 2, 3).reshape(NP, PR, sk)

    return pl.pallas_call(
        kernel,
        out_shape=jax.ShapeDtypeStruct((1, 1, D), A_x.dtype),
        in_specs=[pl.BlockSpec(memory_space=pl.ANY)] * 8,
        scratch_shapes=[
            pltpu.VMEM((NP + 1, 4 * nu, PR // 2, 128), U32),
            pltpu.VMEM((NP, 4 * nu, PR // 2, 128), U32),
            pltpu.VMEM((NP * NC + 1, D // 2, 128), U32),
            pltpu.VMEM((KC, NP + 1, PR // 2, 128), U32),
            pltpu.VMEM((FC, D // 2, 128), U32),
            pltpu.VMEM((FC, D // 2, 128), U32),
            pltpu.VMEM((KC, FF // 2, 128), U32),
            pltpu.VMEM((1, 1, D), BF16),
            pltpu.VMEM((8, D), F32),
            pltpu.VMEM((KC, 8, PR), F32),
            pltpu.VMEM((NC, 8, 128), F32),
            pltpu.VMEM((nu, 8, 128), F32),
            pltpu.VMEM((nu, 8, 128), F32),
            pltpu.VMEM((nu, 8, 128), F32),
            pltpu.VMEM((2, 4 * nu, 8, 128), F32),
            pltpu.VMEM((NP, 8, 128), F32),
            pltpu.VMEM((nu, 8, PR), F32),
            pltpu.VMEM((NC, 8, D), F32),
            pltpu.VMEM((8, D), F32),
            pltpu.SemaphoreType.DMA((NP,)),
            pltpu.SemaphoreType.DMA((NP,)),
            pltpu.SemaphoreType.DMA((5 + W2_CHUNKS,)),
        ],
        compiler_params=pltpu.CompilerParams(
            vmem_limit_bytes=126 * 1024 * 1024, disable_semaphore_checks=True),
        name="interleave_decode",
    )(A_x, as_rows(A_k_cache), as_rows(A_v_cache), A_wq, A_wo.reshape(NP, PR, D),
      B_w1, B_w3, B_w2)
```

```python
import jax
import jax.numpy as jnp
from jax import lax
import jax.experimental.pallas as pl
import jax.experimental.pallas.tpu as pltpu

F32, BF16, U32 = jnp.float32, jnp.bfloat16, jnp.uint32

D, HQ, DH, FF = 640, 32, 192, 1536
NP = HQ // 2
PR = 2 * DH
KC, NC, FC = D // 128, PR // 128, FF // 128
EPS = 1e-5
SCALE = DH ** -0.5

MXU_TILES_STEADY = 2
MXU_TILES_LAST = 16
W2_CHUNKS = 4
FENCE_EVERY = 8
PV_BLOCK = 3
MXU_LEAD = 4


def _bf(w):
    return pltpu.bitcast(w, BF16)


def _mm(lhs, w):
    return lax.dot_general(lhs, _bf(w), (((1,), (0,)), ((), ())),
                           preferred_element_type=F32)


def _mm_t(lhs, w):
    return lax.dot_general(lhs, _bf(w), (((1,), (1,)), ((), ())),
                           preferred_element_type=F32)


def _round(x):
    return x.astype(BF16).astype(F32)


def _tree_sum(xs):
    xs = list(xs)
    while len(xs) > 1:
        xs = [xs[i] + xs[i + 1] if i + 1 < len(xs) else xs[i]
              for i in range(0, len(xs), 2)]
    return xs[0]


def _layernorm(x):
    m = jnp.mean(x, axis=-1, keepdims=True)
    c = x - m
    v = jnp.mean(c * c, axis=-1, keepdims=True)
    return _round(c * lax.rsqrt(v + EPS))


def _interleave(a, na, lead, b, nb):
    ia = ib = 0
    while ia < na or ib < nb:
        if ib >= nb or (ia < na and (ia - lead) * nb <= ib * na):
            ia += next(a)
        else:
            ib += next(b)
    for _ in a:
        pass
    for _ in b:
        pass


def _make_kernel(s0, win):
    nt = win // 128
    nu = nt // 4
    m_steady, m_last = MXU_TILES_STEADY, MXU_TILES_LAST
    T_WO = nt
    T_WQ = T_WO + KC
    T_V = T_WQ + 2 * NC
    n_slots = max(T_V + m_steady, NC + m_last)

    def kernel(x_hbm, k_hbm, v_hbm, wq_hbm, wo_hbm, w1_hbm, w3_hbm, w2_hbm, o_ref,
               mb, vb, w1b, w3b, w2b, xb,
               xn_s, qp, ql, sa, sb, pb, pbb, rl, dg, ox, ol, yp,
               sem_k, sem_v, sem_w):
        row = lax.broadcasted_iota(jnp.int32, (8, 128), 0)
        lane = lax.broadcasted_iota(jnp.int32, (8, 128), 1)

        def group(n, src, buf, idx, sem):
            def copy(i):
                return pltpu.make_async_copy(src(i), buf.bitcast(BF16).at[idx(i)], sem)
            return n, copy

        def col(i, base=0):
            return pl.ds(pl.multiple_of(base + i * 128, 128), 128)

        def start(groups):
            for n, copy in groups:
                lax.fori_loop(0, n, lambda i, c: (copy(i).start(), c)[1], 0)

        def wait(groups):
            for n, copy in groups:
                lax.fori_loop(0, n, lambda i, c: (copy(i).wait(), c)[1], 0)

        def k_copy(g):
            return [group(nt, lambda i: k_hbm.at[g, :, col(i, s0)],
                          mb, lambda i: (g, i), sem_k.at[g])]

        def v_copy(g, m, slot, t0):
            return [group(m, lambda i: v_hbm.at[g, :, col(i, s0)],
                          mb, lambda i: (slot, t0 + i), sem_v.at[g]),
                    group(nt - m, lambda i: v_hbm.at[g, :, col(i, s0 + m * 128)],
                          vb, lambda i: (g, m - m_steady + i), sem_v.at[g])]

        x_copy = pltpu.make_async_copy(x_hbm, xb, sem_w.at[0])
        wq_copy = [
            group(NP * NC, lambda i, r=r, n=n: wq_hbm.at[pl.ds(r, n), col(i)], mb,
                  lambda i, r=r, n=n: (lax.div(i, NC), T_WQ + 2 * lax.rem(i, NC) + r // PR,
                                       pl.ds(0, n)),
                  sem_w.at[1])
            for r, n in ((0, PR), (PR, D - PR))]
        wo_copy = [group(KC, lambda i: wo_hbm.at[:, :, col(i)],
                         mb, lambda i: (pl.ds(0, NP), T_WO + i), sem_w.at[2])]
        w13_copy = [group(FC, lambda i, w=w: w.at[:, col(i)], b, lambda i: (i,), sem_w.at[3])
                    for w, b in ((w1_hbm, w1b), (w3_hbm, w3b))]

        def w2_copy(c):
            rows = pl.ds(c * (FF // W2_CHUNKS), FF // W2_CHUNKS)
            return [group(KC, lambda i: w2_hbm.at[rows, col(i)],
                          w2b, lambda i: (i, rows), sem_w.at[4 + c])]

        start(wo_copy)
        x_copy.start()
        start(wq_copy + k_copy(0))

        def mxu_scores(g):
            lhs = [ql[j] for j in range(NC)]
            for t in range(nt):
                u, r = t // 4, 2 * (t % 4)
                sa[u, r:r + 1, :] = _mm(lhs[0], mb[g, t, 0:64, :])[r:r + 1]
                yield 1
                sb[u, r:r + 2, :] = _mm(lhs[1], mb[g, t, 64:128, :])[r:r + 2]
                yield 1
                sa[u, r + 1:r + 2, :] = _mm(lhs[2], mb[g, t, 128:192, :])[r + 1:r + 2]
                yield 1

        def mxu_q(g):
            for n in range(NC):
                for c in range(KC):
                    r0 = c % NC * 64
                    qp[c, :, n * 128:(n + 1) * 128] = _mm(
                        xn_s[:, c * 128:(c + 1) * 128],
                        mb[g, T_WQ + 2 * n + c // NC, r0:r0 + 64, :])
                    yield 1

        def mxu_wo(g):
            for j in range(NC):
                o = ol[j]
                for n in range(KC):
                    yp[g, j, :, n * 128:(n + 1) * 128] = _mm(
                        o, mb[g, T_WO + n, j * 64:(j + 1) * 64, :])
                    yield 1

        def mxu_pv(m, slot, t0):
            for t in range(m):
                u, r = t // 4, 2 * (t % 4)
                p = pb[u]
                for j in range(NC):
                    ox[u, r:r + 2, j * 128:(j + 1) * 128] = _mm_t(
                        p, mb[slot, t0 + t, j * 64:(j + 1) * 64, :])[r:r + 2]
                    yield 2

        def vpu_pv(g, m):
            pending = []

            def flush():
                for d0, total in pending:
                    j, c0 = divmod(d0, 128)
                    total = jnp.broadcast_to(total, (8, 128))
                    dg[j, :, c0:c0 + 8] = total[:, c0:c0 + 8]
                pending.clear()

            for h in range(2):
                for i0 in range(0, DH // 16, PV_BLOCK):
                    acc = [None] * PV_BLOCK
                    for t in range(m, nt):
                        if i0 == 0:
                            r = 2 * (t % 4) + h
                            p = jnp.broadcast_to(pb[t // 4, r:r + 1, :], (8, 128))
                            pbb[h, t] = p
                        else:
                            p = pbb[h, t]
                        p = jnp.concatenate([p, p], axis=0)
                        for i in range(PV_BLOCK):
                            r0 = h * (DH // 2) + (i0 + i) * 8
                            v = _bf(vb[g, t - m_steady, r0:r0 + 8, :]).astype(F32) * p
                            acc[i] = v if acc[i] is None else acc[i] + v
                        if (nt - 1 - t) % FENCE_EVERY == 0:
                            for i in range(PV_BLOCK):
                                mb[NP, 0, i * 16:(i + 1) * 16, :] = pltpu.bitcast(acc[i], U32)
                        if t == nt - 1:
                            for i in range(PV_BLOCK):
                                for k in (0, 8):
                                    pending.append((
                                        h * DH + (i0 + i) * 16 + k,
                                        jnp.sum(acc[i][k:k + 8], axis=1, keepdims=True)))
                            flush()
                        yield PV_BLOCK
            flush()

        def per_head(x, op):
            x = op(x, pltpu.roll(x, 2, 0))
            return op(x, pltpu.roll(x, 4, 0))

        def q_finish():
            q = _round(_tree_sum(qp[c] for c in range(KC)))
            ql[0] = q[:, :128]
            ql[1] = jnp.where((row & 1) == (lane >> 6), q[:, 128:256], 0.0)
            ql[2] = q[:, 256:]

        def softmax():
            s = [sa[u] + sb[u] for u in range(nu)]
            m = s[0]
            for x in s[1:]:
                m = jnp.maximum(m, x)
            m = jnp.max(per_head(m, jnp.maximum), axis=1, keepdims=True)
            p = [jnp.exp((x - m) * SCALE) for x in s]
            l = jnp.sum(per_head(_tree_sum(p), jnp.add), axis=1, keepdims=True)
            inv = jnp.broadcast_to(1.0 / l, (8, 128))
            inv_o = pltpu.roll(inv, 1, 0)
            even = (row & 1) == 0
            inv_a, inv_b = jnp.where(even, inv, inv_o), jnp.where(even, inv_o, inv)
            for u in range(nu):
                pb[u] = p[u]
            rl[0], rl[1], rl[2] = inv_a, jnp.where(lane < 64, inv_a, inv_b), inv_b

        def pv_finish(m):
            own = ((row & 1) == 0, (row & 1) == (lane >> 6), (row & 1) == 1)
            for j in range(NC):
                part = []
                if m < nt:
                    part.append(jnp.where((lane & 7) == row, dg[j], 0.0))
                if m >= 4:
                    part.append(jnp.where(own[j], _tree_sum(
                        ox[u, :, j * 128:(j + 1) * 128] for u in range(m // 4)), 0.0))
                if m % 4:
                    part.append(jnp.where(jnp.logical_and(own[j], row < 2 * (m % 4)),
                                          ox[m // 4, :, j * 128:(j + 1) * 128], 0.0))
                ol[j] = _round(_tree_sum(part) * rl[j])

        def stage(g, *, q_next, scores, pv, wo):
            mxu, vpu, n_vpu = [], iter(()), 0
            if pv is not None and pv[0] < nt:
                vpu, n_vpu = vpu_pv(g - 1, pv[0]), (nt - pv[0]) * PR // 16
            if scores:
                mxu.append((mxu_scores(g), NC * nt))
            if q_next:
                mxu.append((mxu_q(g + 1), NC * KC))
            if pv is not None:
                mxu.append((mxu_pv(*pv), 2 * NC * pv[0]))
            if wo:
                mxu.append((mxu_wo(g - 2), NC * KC))
            _interleave((w for s, _ in mxu for w in s), sum(n for _, n in mxu),
                        MXU_LEAD, vpu, n_vpu)
            if pv is not None:
                pv_finish(pv[0])
            if scores:
                softmax()
            if q_next:
                q_finish()

        def layer(it, x):
            z = it >> 1

            def first_layer(await_, start_=()):
                @pl.when(it == 0)
                def _():
                    start(start_)
                    wait(await_)

            def pv(g):
                return m_steady, g, T_V

            def v_steady(g):
                return v_copy(g, *pv(g))

            pv_last = (m_last, NP + z, NC)
            v_last = v_copy(NP - 1, *pv_last)

            xn_s[...] = _layernorm(x)
            dg[...] = jnp.zeros_like(dg)
            first_layer(wo_copy + wq_copy + k_copy(0), k_copy(1) + v_steady(0))
            for _ in mxu_q(0):
                pass
            q_finish()
            stage(z, q_next=True, scores=True, pv=None, wo=False)
            first_layer(k_copy(1) + v_steady(0), k_copy(2) + v_steady(1))
            stage(1 + z, q_next=True, scores=True, pv=pv(z), wo=False)

            def body(g, carry):
                first_layer(k_copy(g) + v_steady(g - 1), k_copy(g + 1) + v_steady(g))
                stage(g, q_next=True, scores=True, pv=pv(g - 1), wo=True)
                return carry

            lax.fori_loop(2, NP - 1, body, 0)
            first_layer(k_copy(NP - 1) + v_steady(NP - 2), v_last)
            stage(NP - 1 + z, q_next=False, scores=True, pv=pv(NP - 2 + z),
                  wo=True)
            first_layer(v_last, w13_copy + sum((w2_copy(c) for c in range(W2_CHUNKS)), []))
            stage(NP + z, q_next=False, scores=False, pv=pv_last, wo=True)
            stage(NP + 1, q_next=False, scores=False, pv=None, wo=True)
            y = yp[0, 0]
            for i in range(1, NP * NC):
                y = y + yp[i // NC, i % NC]
            x = _round(x + _round(jnp.sum(y, axis=0, keepdims=True)))

            xn = _layernorm(x)
            first_layer(w13_copy)
            h = []
            for f in range(FC):
                gate, up = (
                    _round(_tree_sum(
                        _mm(xn[:, c * 128:(c + 1) * 128], w[f, c * 64:(c + 1) * 64, :])
                        for c in range(KC)))
                    for w in (w1b, w3b))
                h.append(_round(_round(gate * jax.nn.sigmoid(gate)) * up))
            y = [None] * KC
            per = FC // W2_CHUNKS
            for c in range(W2_CHUNKS):
                first_layer(w2_copy(c))
                for f in range(c * per, (c + 1) * per):
                    for n in range(KC):
                        r = _mm(h[f], w2b[n, f * 64:(f + 1) * 64, :])
                        y[n] = r if y[n] is None else y[n] + r
            return _round(x + _round(jnp.concatenate(y, axis=1)))

        x_copy.wait()
        x = jnp.broadcast_to(xb[0].astype(F32), (8, D))
        x = lax.fori_loop(0, 2, layer, x)
        o_ref[0] = x[0:1].astype(o_ref.dtype)

    return kernel, nu, n_slots


@jax.jit
def pallas_interleave_layers__sliding_block_cached__glu_gated_swiglu__decode_kernel(
    A_x: jax.Array,
    A_k_cache: jax.Array,
    A_v_cache: jax.Array,
    A_wq: jax.Array,
    A_wo: jax.Array,
    B_x: jax.Array,
    B_w1: jax.Array,
    B_w3: jax.Array,
    B_w2: jax.Array,
):
    del B_x
    sk = A_k_cache.shape[2]
    win = min(4096, max(256, sk // 4))
    assert A_x.shape == (1, 1, D) and A_k_cache.shape == (1, HQ, sk, DH)
    assert win % 1024 == 0 and (sk - win) % 128 == 0
    kernel, nu, n_slots = _make_kernel(sk - win, win)

    def as_rows(c):
        return jnp.swapaxes(c, 2, 3).reshape(NP, PR, sk)

    return pl.pallas_call(
        kernel,
        out_shape=jax.ShapeDtypeStruct((1, 1, D), A_x.dtype),
        in_specs=[pl.BlockSpec(memory_space=pl.ANY)] * 8,
        scratch_shapes=[
            pltpu.VMEM((NP + 1, n_slots, PR // 2, 128), U32),
            pltpu.VMEM((NP, 4 * nu - MXU_TILES_STEADY, PR // 2, 128), U32),
            pltpu.VMEM((FC, D // 2, 128), U32),
            pltpu.VMEM((FC, D // 2, 128), U32),
            pltpu.VMEM((KC, FF // 2, 128), U32),
            pltpu.VMEM((1, 1, D), BF16),
            pltpu.VMEM((8, D), F32),
            pltpu.VMEM((KC, 8, PR), F32),
            pltpu.VMEM((NC, 8, 128), F32),
            pltpu.VMEM((nu, 8, 128), F32),
            pltpu.VMEM((nu, 8, 128), F32),
            pltpu.VMEM((nu, 8, 128), F32),
            pltpu.VMEM((2, 4 * nu, 8, 128), F32),
            pltpu.VMEM((NC, 8, 128), F32),
            pltpu.VMEM((NC, 8, 128), F32),
            pltpu.VMEM((nu, 8, PR), F32),
            pltpu.VMEM((NC, 8, 128), F32),
            pltpu.VMEM((NP, NC, 8, D), F32),
            pltpu.SemaphoreType.DMA((NP,)),
            pltpu.SemaphoreType.DMA((NP,)),
            pltpu.SemaphoreType.DMA((4 + W2_CHUNKS,)),
        ],
        compiler_params=pltpu.CompilerParams(
            vmem_limit_bytes=128 * 1024 * 1024, disable_semaphore_checks=True),
        name="interleave_decode",
    )(A_x, as_rows(A_k_cache), as_rows(A_v_cache), A_wq, A_wo.reshape(NP, PR, D),
      B_w1, B_w3, B_w2)
```

```python
import jax
import jax.numpy as jnp
from jax import lax
import jax.experimental.pallas as pl
import jax.experimental.pallas.tpu as pltpu

F32, BF16, U32 = jnp.float32, jnp.bfloat16, jnp.uint32

D, HQ, DH, FF = 640, 32, 192, 1536
NP = HQ // 2
PR = 2 * DH
KC, NC, FC = D // 128, PR // 128, FF // 128
EPS = 1e-5
SCALE = DH ** -0.5

MXU_TILES_STEADY = 2
MXU_TILES_LAST = 12
W2_CHUNKS = (8, 3, 1)
MXU_SLACK = 0
ORDER = 'qvo'
ONLY_LOOP = False
FENCE_EVERY = 8
PV_BLOCK = 3
MXU_LEAD = 4


def _bf(w):
    return pltpu.bitcast(w, BF16)


def _mm(lhs, w):
    return lax.dot_general(lhs, _bf(w), (((1,), (0,)), ((), ())),
                           preferred_element_type=F32)


def _mm_t(lhs, w):
    return lax.dot_general(lhs, _bf(w), (((1,), (1,)), ((), ())),
                           preferred_element_type=F32)


def _round(x):
    return x.astype(BF16).astype(F32)


def _tree_sum(xs):
    xs = list(xs)
    while len(xs) > 1:
        xs = [xs[i] + xs[i + 1] if i + 1 < len(xs) else xs[i]
              for i in range(0, len(xs), 2)]
    return xs[0]


def _layernorm(x):
    xs = [x[:, c * 128:(c + 1) * 128] for c in range(KC)]
    c = x - jnp.sum(_tree_sum(xs), axis=-1, keepdims=True) * (1.0 / D)
    sq = _tree_sum(c[:, i * 128:(i + 1) * 128] ** 2 for i in range(KC))
    v = jnp.sum(sq, axis=-1, keepdims=True) * (1.0 / D)
    return _round(c), jnp.broadcast_to(lax.rsqrt(v + EPS), (8, 128))


def _interleave(a, na, lead, b, nb):
    ia = ib = 0
    for w in b:
        ib += w
        while (ia - lead) * nb < ib * na:
            ia += next(a, na)
    for _ in a:
        pass


def _make_kernel(s0, win):
    nt = win // 128
    nu = nt // 4
    m_steady, m_last = MXU_TILES_STEADY, MXU_TILES_LAST
    T_WO = nt
    T_WQ = T_WO + KC
    T_V = T_WQ + 2 * NC
    n_slots = max(T_V + m_steady, NC + m_last)

    def kernel(x_hbm, k_hbm, v_hbm, wq_hbm, wo_hbm, w1_hbm, w3_hbm, w2_hbm, o_ref,
               mb, vb, w1b, w3b, w2b, xb,
               xs, xn_s, xf, qp, ql, sa, sb, pb, pbb, rl, dg, ox, ol, yp,
               sem_k, sem_v, sem_w):
        row = lax.broadcasted_iota(jnp.int32, (8, 128), 0)
        lane = lax.broadcasted_iota(jnp.int32, (8, 128), 1)

        def group(n, src, buf, idx, sem):
            def copy(i):
                return pltpu.make_async_copy(src(i), buf.bitcast(BF16).at[idx(i)], sem)
            return n, copy

        def col(i, base=0):
            return pl.ds(pl.multiple_of(base + i * 128, 128), 128)

        def start(groups):
            for n, copy in groups:
                lax.fori_loop(0, n, lambda i, c: (copy(i).start(), c)[1], 0)

        def wait(groups):
            for n, copy in groups:
                lax.fori_loop(0, n, lambda i, c: (copy(i).wait(), c)[1], 0)

        def k_copy(g):
            return [group(nt, lambda i: k_hbm.at[g, :, col(i, s0)],
                          mb, lambda i: (g, i), sem_k.at[g])]

        def v_copy(g, m, slot, t0):
            return [group(m, lambda i: v_hbm.at[g, :, col(i, s0)],
                          mb, lambda i: (slot, t0 + i), sem_v.at[g]),
                    group(nt - m, lambda i: v_hbm.at[g, :, col(i, s0 + m * 128)],
                          vb, lambda i: (g, m - m_steady + i), sem_v.at[g])]

        x_copy = pltpu.make_async_copy(x_hbm, xb, sem_w.at[0])
        wq_copy = [
            group(NP * NC, lambda i, r=r, n=n: wq_hbm.at[pl.ds(r, n), col(i)], mb,
                  lambda i, r=r, n=n: (lax.div(i, NC), T_WQ + 2 * lax.rem(i, NC) + r // PR,
                                       pl.ds(0, n)),
                  sem_w.at[1])
            for r, n in ((0, PR), (PR, D - PR))]
        wo_copy = [group(KC, lambda i: wo_hbm.at[:, :, col(i)],
                         mb, lambda i: (pl.ds(0, NP), T_WO + i), sem_w.at[2])]
        w13_copy = [group(FC, lambda i, w=w: w.at[:, col(i)], b, lambda i: (i,), sem_w.at[3])
                    for w, b in ((w1_hbm, w1b), (w3_hbm, w3b))]

        def w2_copy(c):
            rows = pl.ds(128 * sum(W2_CHUNKS[:c]), 128 * W2_CHUNKS[c])
            return [group(KC, lambda i: w2_hbm.at[rows, col(i)],
                          w2b, lambda i: (i, rows), sem_w.at[4 + c])]

        start(wo_copy)
        x_copy.start()
        start(wq_copy + k_copy(0))

        def mxu_scores(g):
            lhs = [ql[j] for j in range(NC)]
            for t in range(nt):
                u, r = t // 4, 2 * (t % 4)
                sa[u, r:r + 1, :] = _mm(lhs[0], mb[g, t, 0:64, :])[r:r + 1]
                yield 1
                sb[u, r:r + 2, :] = _mm(lhs[1], mb[g, t, 64:128, :])[r:r + 2]
                yield 1
                sa[u, r + 1:r + 2, :] = _mm(lhs[2], mb[g, t, 128:192, :])[r + 1:r + 2]
                yield 1

        def mxu_q(g, slot=0):
            for n in range(NC):
                for c in range(KC):
                    r0 = c % NC * 64
                    qp[slot, c, :, n * 128:(n + 1) * 128] = _mm(
                        xn_s[:, c * 128:(c + 1) * 128],
                        mb[g, T_WQ + 2 * n + c // NC, r0:r0 + 64, :])
                    yield 1

        def mxu_wo(g):
            for j in range(NC):
                o = ol[j]
                for n in range(KC):
                    yp[g, j, :, n * 128:(n + 1) * 128] = _mm(
                        o, mb[g, T_WO + n, j * 64:(j + 1) * 64, :])
                    yield 1

        def mxu_pv(m, slot, t0):
            for t in range(m):
                u, r = t // 4, 2 * (t % 4)
                p = pb[u]
                for j in range(NC):
                    ox[u, r:r + 2, j * 128:(j + 1) * 128] = _mm_t(
                        p, mb[slot, t0 + t, j * 64:(j + 1) * 64, :])[r:r + 2]
                    yield 2

        def vpu_pv(g, m):
            pending = []

            def flush():
                for d0, total in pending:
                    j, c0 = divmod(d0, 128)
                    total = jnp.broadcast_to(total, (8, 128))
                    dg[j, :, c0:c0 + 8] = total[:, c0:c0 + 8]
                pending.clear()

            for h in range(2):
                for i0 in range(0, DH // 16, PV_BLOCK):
                    acc = [None] * PV_BLOCK
                    for t in range(m, nt):
                        if i0 == 0:
                            r = 2 * (t % 4) + h
                            p = jnp.broadcast_to(pb[t // 4, r:r + 1, :], (8, 128))
                            pbb[h, t] = p
                        else:
                            p = pbb[h, t]
                        p = jnp.concatenate([p, p], axis=0)
                        for i in range(PV_BLOCK):
                            r0 = h * (DH // 2) + (i0 + i) * 8
                            v = _bf(vb[g, t - m_steady, r0:r0 + 8, :]).astype(F32) * p
                            acc[i] = v if acc[i] is None else acc[i] + v
                        if (nt - 1 - t) % FENCE_EVERY == 0:
                            for i in range(PV_BLOCK):
                                mb[NP, 0, i * 16:(i + 1) * 16, :] = pltpu.bitcast(acc[i], U32)
                        if t == nt - 1:
                            for i in range(PV_BLOCK):
                                for k in (0, 8):
                                    pending.append((
                                        h * DH + (i0 + i) * 16 + k,
                                        jnp.sum(acc[i][k:k + 8], axis=1, keepdims=True)))
                            flush()
                        yield PV_BLOCK
            flush()

        def per_head(x, op):
            x = op(x, pltpu.roll(x, 2, 0))
            return op(x, pltpu.roll(x, 4, 0))

        def q_finish(slot=0):
            q = _tree_sum(qp[slot, c] for c in range(KC))
            q = _round(q * jnp.concatenate([xf[...]] * NC, axis=1))
            ql[0] = q[:, :128]
            ql[1] = jnp.where((row & 1) == (lane >> 6), q[:, 128:256], 0.0)
            ql[2] = q[:, 256:]

        def softmax():
            s = [sa[u] + sb[u] for u in range(nu)]
            m = s[0]
            for x in s[1:]:
                m = jnp.maximum(m, x)
            m = jnp.max(per_head(m, jnp.maximum), axis=1, keepdims=True)
            p = [jnp.exp((x - m) * SCALE) for x in s]
            l = jnp.sum(per_head(_tree_sum(p), jnp.add), axis=1, keepdims=True)
            inv = jnp.broadcast_to(1.0 / l, (8, 128))
            inv_o = pltpu.roll(inv, 1, 0)
            even = (row & 1) == 0
            inv_a, inv_b = jnp.where(even, inv, inv_o), jnp.where(even, inv_o, inv)
            for u in range(nu):
                pb[u] = p[u]
            rl[0], rl[1], rl[2] = inv_a, jnp.where(lane < 64, inv_a, inv_b), inv_b

        def pv_finish(m):
            own = ((row & 1) == 0, (row & 1) == (lane >> 6), (row & 1) == 1)
            for j in range(NC):
                part = []
                if m < nt:
                    part.append(jnp.where((lane & 7) == row, dg[j], 0.0))
                if m >= 4:
                    part.append(jnp.where(own[j], _tree_sum(
                        ox[u, :, j * 128:(j + 1) * 128] for u in range(m // 4)), 0.0))
                if m % 4:
                    part.append(jnp.where(jnp.logical_and(own[j], row < 2 * (m % 4)),
                                          ox[m // 4, :, j * 128:(j + 1) * 128], 0.0))
                ol[j] = _round(_tree_sum(part) * rl[j])

        def stage(g, *, q_next, scores, pv, wo):
            mxu, vpu, n_vpu = [], iter(()), 0
            if ONLY_LOOP and not (q_next and wo):
                return
            if pv is not None and pv[0] < nt:
                vpu, n_vpu = vpu_pv(g - 1, pv[0]), (nt - pv[0]) * PR // 16
            if scores:
                mxu.append((mxu_scores(g), NC * nt))
            part = {"q": q_next and pv and (mxu_q(g + 1), NC * KC),
                    "v": pv and (mxu_pv(*pv), 2 * NC * pv[0]),
                    "o": wo and (mxu_wo(g - 2), NC * KC)}
            mxu += [part[k] for k in ORDER if part[k]]
            _interleave((w for s, _ in mxu for w in s), sum(n for _, n in mxu) + MXU_SLACK,
                        MXU_LEAD, vpu, n_vpu)
            if pv is not None:
                pv_finish(pv[0])
            if scores:
                softmax()
            if q_next:
                q_finish()

        def run(stream):
            for _ in stream:
                pass

        def ffn(x, loading):
            xn, factor = _layernorm(x)
            if loading:
                wait(w13_copy)
            h = []
            for f in range(FC):
                gate, up = (
                    _round(factor * _tree_sum(
                        _mm(xn[:, c * 128:(c + 1) * 128], w[f, c * 64:(c + 1) * 64, :])
                        for c in range(KC)))
                    for w in (w1b, w3b))
                h.append(_round(_round(gate * jax.nn.sigmoid(gate)) * up))
            y = [None] * KC
            for c, size in enumerate(W2_CHUNKS):
                if loading:
                    wait(w2_copy(c))
                for f in range(sum(W2_CHUNKS[:c]), sum(W2_CHUNKS[:c + 1])):
                    for n in range(KC):
                        r = _mm(h[f], w2b[n, f * 64:(f + 1) * 64, :])
                        y[n] = r if y[n] is None else y[n] + r
            xs[...] = _round(x + _round(jnp.concatenate(y, axis=1)))

        def layer(it, carry):
            z = it >> 1

            def first_layer(await_, start_=()):
                @pl.when(it == 0)
                def _():
                    start(start_)
                    wait(await_)

            def pv(g):
                return m_steady, g, T_V

            def v_steady(g):
                return v_copy(g, *pv(g))

            pv_last = (m_last, NP + z, NC)
            v_last = v_copy(NP - 1, *pv_last)

            first_layer(wo_copy + wq_copy + k_copy(0), k_copy(1) + v_steady(0))
            xn_s[...], xf[...] = _layernorm(xs[...])
            run(mxu_q(0, 1))
            run(mxu_q(1))
            q_finish(1)
            stage(z, q_next=True, scores=True, pv=None, wo=False)
            first_layer(k_copy(1) + v_steady(0), k_copy(2) + v_steady(1))
            stage(1 + z, q_next=True, scores=True, pv=pv(z), wo=False)

            def body(g, carry):
                first_layer(k_copy(g) + v_steady(g - 1), k_copy(g + 1) + v_steady(g))
                stage(g, q_next=True, scores=True, pv=pv(g - 1), wo=True)
                return carry

            lax.fori_loop(2, NP - 1, body, 0)
            first_layer(k_copy(NP - 1) + v_steady(NP - 2), v_last)
            stage(NP - 1 + z, q_next=False, scores=True, pv=pv(NP - 2 + z), wo=True)
            first_layer(v_last, w13_copy + sum((w2_copy(c) for c in range(len(W2_CHUNKS))), []))
            y = yp[0, 0]
            for i in range(1, (NP - 2) * NC):
                y = y + yp[i // NC, i % NC]
            yp[0, 0] = y
            stage(NP + z, q_next=False, scores=False, pv=pv_last, wo=True)
            run(mxu_wo(NP - 1))
            y = _tree_sum(yp[g, j] for g, j in
                          [(0, 0)] + [(g, j) for g in (NP - 2, NP - 1) for j in range(NC)])
            xs[...] = _round(xs[...] + _round(jnp.sum(y, axis=0, keepdims=True)))
            pl.when(it == 0)(lambda: ffn(xs[...], True))
            pl.when(it != 0)(lambda: ffn(xs[...], False))
            return carry

        dg[...] = jnp.zeros_like(dg)
        x_copy.wait()
        xs[...] = jnp.broadcast_to(xb[0].astype(F32), (8, D))
        lax.fori_loop(0, 2, layer, 0)
        o_ref[0] = xs[0:1, :].astype(o_ref.dtype)

    return kernel, nu, n_slots


@jax.jit
def pallas_interleave_layers__sliding_block_cached__glu_gated_swiglu__decode_kernel(
    A_x: jax.Array,
    A_k_cache: jax.Array,
    A_v_cache: jax.Array,
    A_wq: jax.Array,
    A_wo: jax.Array,
    B_x: jax.Array,
    B_w1: jax.Array,
    B_w3: jax.Array,
    B_w2: jax.Array,
):
    del B_x
    sk = A_k_cache.shape[2]
    win = min(4096, max(256, sk // 4))
    assert A_x.shape == (1, 1, D) and A_k_cache.shape == (1, HQ, sk, DH)
    assert win % 1024 == 0 and (sk - win) % 128 == 0
    kernel, nu, n_slots = _make_kernel(sk - win, win)

    def as_rows(c):
        return jnp.swapaxes(c, 2, 3).reshape(NP, PR, sk)

    return pl.pallas_call(
        kernel,
        out_shape=jax.ShapeDtypeStruct((1, 1, D), A_x.dtype),
        in_specs=[pl.BlockSpec(memory_space=pl.ANY)] * 8,
        scratch_shapes=[
            pltpu.VMEM((NP + 1, n_slots, PR // 2, 128), U32),
            pltpu.VMEM((NP, 4 * nu - MXU_TILES_STEADY, PR // 2, 128), U32),
            pltpu.VMEM((FC, D // 2, 128), U32),
            pltpu.VMEM((FC, D // 2, 128), U32),
            pltpu.VMEM((KC, FF // 2, 128), U32),
            pltpu.VMEM((1, 1, D), BF16),
            pltpu.VMEM((8, D), F32),
            pltpu.VMEM((8, D), F32),
            pltpu.VMEM((8, 128), F32),
            pltpu.VMEM((2, KC, 8, PR), F32),
            pltpu.VMEM((NC, 8, 128), F32),
            pltpu.VMEM((nu, 8, 128), F32),
            pltpu.VMEM((nu, 8, 128), F32),
            pltpu.VMEM((nu, 8, 128), F32),
            pltpu.VMEM((2, 4 * nu, 8, 128), F32),
            pltpu.VMEM((NC, 8, 128), F32),
            pltpu.VMEM((NC, 8, 128), F32),
            pltpu.VMEM((nu, 8, PR), F32),
            pltpu.VMEM((NC, 8, 128), F32),
            pltpu.VMEM((NP, NC, 8, D), F32),
            pltpu.SemaphoreType.DMA((NP,)),
            pltpu.SemaphoreType.DMA((NP,)),
            pltpu.SemaphoreType.DMA((4 + len(W2_CHUNKS),)),
        ],
        compiler_params=pltpu.CompilerParams(
            vmem_limit_bytes=128 * 1024 * 1024, disable_semaphore_checks=True),
        name="interleave_decode",
    )(A_x, as_rows(A_k_cache), as_rows(A_v_cache), A_wq, A_wo.reshape(NP, PR, D),
      B_w1, B_w3, B_w2)
```

```python
import jax
import jax.numpy as jnp
from jax import lax
import jax.experimental.pallas as pl
import jax.experimental.pallas.tpu as pltpu

F32, BF16, U32 = jnp.float32, jnp.bfloat16, jnp.uint32

D, HQ, DH, FF = 640, 32, 192, 1536
NP = HQ // 2
PR = 2 * DH
KC, NC, FC = D // 128, PR // 128, FF // 128
EPS = 1e-5
SCALE = DH ** -0.5

MXU_TILES_STEADY = 2
MXU_TILES_LAST = 12
W2_CHUNKS = (8, 3, 1)
MXU_SLACK = 0
ORDER = 'qvo'
ONLY_LOOP = False
FENCE_EVERY = 8
PV_BLOCK = 3
MXU_LEAD = 4


def _bf(w):
    return pltpu.bitcast(w, BF16)


def _mm(lhs, w):
    return lax.dot_general(lhs, _bf(w), (((1,), (0,)), ((), ())),
                           preferred_element_type=F32)


def _mm_t(lhs, w):
    return lax.dot_general(lhs, _bf(w), (((1,), (1,)), ((), ())),
                           preferred_element_type=F32)


def _round(x):
    return x.astype(BF16).astype(F32)


def _tree_sum(xs):
    xs = list(xs)
    while len(xs) > 1:
        xs = [xs[i] + xs[i + 1] if i + 1 < len(xs) else xs[i]
              for i in range(0, len(xs), 2)]
    return xs[0]


def _layernorm(x):
    xs = [x[:, c * 128:(c + 1) * 128] for c in range(KC)]
    c = x - jnp.sum(_tree_sum(xs), axis=-1, keepdims=True) * (1.0 / D)
    sq = _tree_sum(c[:, i * 128:(i + 1) * 128] ** 2 for i in range(KC))
    v = jnp.sum(sq, axis=-1, keepdims=True) * (1.0 / D)
    return _round(c), jnp.broadcast_to(lax.rsqrt(v + EPS), (8, 128))


def _interleave(a, na, lead, b, nb):
    ia = ib = 0
    for w in b:
        ib += w
        while (ia - lead) * nb < ib * na:
            ia += next(a, na)
    for _ in a:
        pass


def _make_kernel(s0, win):
    nt = win // 128
    nu = nt // 4
    m_steady, m_last = MXU_TILES_STEADY, MXU_TILES_LAST
    T_WO = nt
    T_WQ = T_WO + KC
    T_V = T_WQ + 2 * NC
    n_slots = max(T_V + m_steady, NC + m_last)

    def kernel(x_hbm, k_hbm, v_hbm, wq_hbm, wo_hbm, w1_hbm, w3_hbm, w2_hbm, o_ref,
               mb, vb, w1b, w3b, w2b, xb,
               xs, xn_s, xf, qp, ql, sa, sb, pb, pbb, rl, dg, ox, ol, yp,
               sem_k, sem_v, sem_w):
        row = lax.broadcasted_iota(jnp.int32, (8, 128), 0)
        lane = lax.broadcasted_iota(jnp.int32, (8, 128), 1)

        def group(n, src, buf, idx, sem):
            def copy(i):
                return pltpu.make_async_copy(src(i), buf.bitcast(BF16).at[idx(i)], sem)
            return n, copy

        def col(i, base=0):
            return pl.ds(pl.multiple_of(base + i * 128, 128), 128)

        def start(groups):
            for n, copy in groups:
                lax.fori_loop(0, n, lambda i, c: (copy(i).start(), c)[1], 0)

        def wait(groups):
            for n, copy in groups:
                lax.fori_loop(0, n, lambda i, c: (copy(i).wait(), c)[1], 0)

        def k_copy(g):
            return [group(nt, lambda i: k_hbm.at[g, :, col(i, s0)],
                          mb, lambda i: (g, i), sem_k.at[g])]

        def v_copy(g, m, slot, t0):
            return [group(m, lambda i: v_hbm.at[g, :, col(i, s0)],
                          mb, lambda i: (slot, t0 + i), sem_v.at[g]),
                    group(nt - m, lambda i: v_hbm.at[g, :, col(i, s0 + m * 128)],
                          vb, lambda i: (g, m - m_steady + i), sem_v.at[g])]

        x_copy = pltpu.make_async_copy(x_hbm, xb, sem_w.at[0])

        def rows(r, n=128):
            return pl.ds(pl.multiple_of(r * n, n), n)

        def tiles(src, r0, n_rows, n_cols, buf, idx, sem):
            def at(i):
                return r0 + lax.div(i, n_cols), lax.rem(i, n_cols)
            return group(n_rows * n_cols, lambda i: src.at[rows(at(i)[0]), col(at(i)[1])],
                         buf, lambda i: idx(*at(i)), sem)

        wq_copy = [
            group(NP * NC, lambda i, c=c: wq_hbm.at[pl.ds(c * 128, 128), col(i)], mb,
                  lambda i, c=c: (lax.div(i, NC), T_WQ + 2 * lax.rem(i, NC) + c // NC,
                                  pl.ds(c % NC * 128, 128)),
                  sem_w.at[1])
            for c in range(KC)]
        wo_copy = [group(NP * KC,
                         lambda i: wo_hbm.at[lax.div(i, KC), :, col(lax.rem(i, KC))], mb,
                         lambda i: (lax.div(i, KC), T_WO + lax.rem(i, KC)), sem_w.at[2])]
        w13_copy = [tiles(w, 0, KC, FC, b, lambda r, c: (c, rows(r)), sem_w.at[3])
                    for w, b in ((w1_hbm, w1b), (w3_hbm, w3b))]

        def w2_copy(c):
            return [tiles(w2_hbm, sum(W2_CHUNKS[:c]), W2_CHUNKS[c], KC, w2b,
                          lambda r, c: (c, rows(r)), sem_w.at[4 + c])]

        start(wo_copy)
        x_copy.start()
        start(wq_copy + k_copy(0))

        def mxu_scores(g):
            lhs = [ql[j] for j in range(NC)]
            for t in range(nt):
                u, r = t // 4, 2 * (t % 4)
                sa[u, r:r + 1, :] = _mm(lhs[0], mb[g, t, 0:64, :])[r:r + 1]
                yield 1
                sb[u, r:r + 2, :] = _mm(lhs[1], mb[g, t, 64:128, :])[r:r + 2]
                yield 1
                sa[u, r + 1:r + 2, :] = _mm(lhs[2], mb[g, t, 128:192, :])[r + 1:r + 2]
                yield 1

        def mxu_q(g, slot=0):
            for n in range(NC):
                for c in range(KC):
                    r0 = c % NC * 64
                    qp[slot, c, :, n * 128:(n + 1) * 128] = _mm(
                        xn_s[:, c * 128:(c + 1) * 128],
                        mb[g, T_WQ + 2 * n + c // NC, r0:r0 + 64, :])
                    yield 1

        def mxu_wo(g):
            for j in range(NC):
                o = ol[j]
                for n in range(KC):
                    yp[g, j, :, n * 128:(n + 1) * 128] = _mm(
                        o, mb[g, T_WO + n, j * 64:(j + 1) * 64, :])
                    yield 1

        def mxu_pv(m, slot, t0):
            for t in range(m):
                u, r = t // 4, 2 * (t % 4)
                p = pb[u]
                for j in range(NC):
                    ox[u, r:r + 2, j * 128:(j + 1) * 128] = _mm_t(
                        p, mb[slot, t0 + t, j * 64:(j + 1) * 64, :])[r:r + 2]
                    yield 2

        def vpu_pv(g, m):
            pending = []

            def flush():
                for d0, total in pending:
                    j, c0 = divmod(d0, 128)
                    total = jnp.broadcast_to(total, (8, 128))
                    dg[j, :, c0:c0 + 8] = total[:, c0:c0 + 8]
                pending.clear()

            for h in range(2):
                for i0 in range(0, DH // 16, PV_BLOCK):
                    acc = [None] * PV_BLOCK
                    for t in range(m, nt):
                        if i0 == 0:
                            r = 2 * (t % 4) + h
                            p = jnp.broadcast_to(pb[t // 4, r:r + 1, :], (8, 128))
                            pbb[h, t] = p
                        else:
                            p = pbb[h, t]
                        p = jnp.concatenate([p, p], axis=0)
                        for i in range(PV_BLOCK):
                            r0 = h * (DH // 2) + (i0 + i) * 8
                            v = _bf(vb[g, t - m_steady, r0:r0 + 8, :]).astype(F32) * p
                            acc[i] = v if acc[i] is None else acc[i] + v
                        if (nt - 1 - t) % FENCE_EVERY == 0:
                            for i in range(PV_BLOCK):
                                mb[NP, 0, i * 16:(i + 1) * 16, :] = pltpu.bitcast(acc[i], U32)
                        if t == nt - 1:
                            for i in range(PV_BLOCK):
                                for k in (0, 8):
                                    pending.append((
                                        h * DH + (i0 + i) * 16 + k,
                                        jnp.sum(acc[i][k:k + 8], axis=1, keepdims=True)))
                            flush()
                        yield PV_BLOCK
            flush()

        def per_head(x, op):
            x = op(x, pltpu.roll(x, 2, 0))
            return op(x, pltpu.roll(x, 4, 0))

        def q_finish(slot=0):
            q = _tree_sum(qp[slot, c] for c in range(KC))
            q = _round(q * jnp.concatenate([xf[...]] * NC, axis=1))
            ql[0] = q[:, :128]
            ql[1] = jnp.where((row & 1) == (lane >> 6), q[:, 128:256], 0.0)
            ql[2] = q[:, 256:]

        def softmax():
            s = [sa[u] + sb[u] for u in range(nu)]
            m = s[0]
            for x in s[1:]:
                m = jnp.maximum(m, x)
            m = jnp.max(per_head(m, jnp.maximum), axis=1, keepdims=True)
            p = [jnp.exp((x - m) * SCALE) for x in s]
            l = jnp.sum(per_head(_tree_sum(p), jnp.add), axis=1, keepdims=True)
            inv = jnp.broadcast_to(1.0 / l, (8, 128))
            inv_o = pltpu.roll(inv, 1, 0)
            even = (row & 1) == 0
            inv_a, inv_b = jnp.where(even, inv, inv_o), jnp.where(even, inv_o, inv)
            for u in range(nu):
                pb[u] = p[u]
            rl[0], rl[1], rl[2] = inv_a, jnp.where(lane < 64, inv_a, inv_b), inv_b

        def pv_finish(m):
            own = ((row & 1) == 0, (row & 1) == (lane >> 6), (row & 1) == 1)
            for j in range(NC):
                part = []
                if m < nt:
                    part.append(jnp.where((lane & 7) == row, dg[j], 0.0))
                if m >= 4:
                    part.append(jnp.where(own[j], _tree_sum(
                        ox[u, :, j * 128:(j + 1) * 128] for u in range(m // 4)), 0.0))
                if m % 4:
                    part.append(jnp.where(jnp.logical_and(own[j], row < 2 * (m % 4)),
                                          ox[m // 4, :, j * 128:(j + 1) * 128], 0.0))
                ol[j] = _round(_tree_sum(part) * rl[j])

        def stage(g, *, q_next, scores, pv, wo):
            mxu, vpu, n_vpu = [], iter(()), 0
            if ONLY_LOOP and not (q_next and wo):
                return
            if pv is not None and pv[0] < nt:
                vpu, n_vpu = vpu_pv(g - 1, pv[0]), (nt - pv[0]) * PR // 16
            if scores:
                mxu.append((mxu_scores(g), NC * nt))
            part = {"q": q_next and pv and (mxu_q(g + 1), NC * KC),
                    "v": pv and (mxu_pv(*pv), 2 * NC * pv[0]),
                    "o": wo and (mxu_wo(g - 2), NC * KC)}
            mxu += [part[k] for k in ORDER if part[k]]
            _interleave((w for s, _ in mxu for w in s), sum(n for _, n in mxu) + MXU_SLACK,
                        MXU_LEAD, vpu, n_vpu)
            if pv is not None:
                pv_finish(pv[0])
            if scores:
                softmax()
            if q_next:
                q_finish()

        def run(stream):
            for _ in stream:
                pass

        def ffn(x, loading):
            xn, factor = _layernorm(x)
            if loading:
                wait(w13_copy)
            h = []
            for f in range(FC):
                gate, up = (
                    _round(factor * _tree_sum(
                        _mm(xn[:, c * 128:(c + 1) * 128], w[f, c * 64:(c + 1) * 64, :])
                        for c in range(KC)))
                    for w in (w1b, w3b))
                h.append(_round(_round(gate * jax.nn.sigmoid(gate)) * up))
            y = [None] * KC
            for c, size in enumerate(W2_CHUNKS):
                if loading:
                    wait(w2_copy(c))
                for f in range(sum(W2_CHUNKS[:c]), sum(W2_CHUNKS[:c + 1])):
                    for n in range(KC):
                        r = _mm(h[f], w2b[n, f * 64:(f + 1) * 64, :])
                        y[n] = r if y[n] is None else y[n] + r
            xs[...] = _round(x + _round(jnp.concatenate(y, axis=1)))

        def layer(it, carry):
            z = it >> 1

            def first_layer(await_, start_=()):
                @pl.when(it == 0)
                def _():
                    start(start_)
                    wait(await_)

            def pv(g):
                return m_steady, g, T_V

            def v_steady(g):
                return v_copy(g, *pv(g))

            pv_last = (m_last, NP + z, NC)
            v_last = v_copy(NP - 1, *pv_last)

            first_layer(wo_copy + wq_copy + k_copy(0), k_copy(1) + v_steady(0))
            xn_s[...], xf[...] = _layernorm(xs[...])
            run(mxu_q(0, 1))
            run(mxu_q(1))
            q_finish(1)
            stage(z, q_next=True, scores=True, pv=None, wo=False)
            first_layer(k_copy(1) + v_steady(0), k_copy(2) + v_steady(1))
            stage(1 + z, q_next=True, scores=True, pv=pv(z), wo=False)

            def body(g, carry):
                first_layer(k_copy(g) + v_steady(g - 1), k_copy(g + 1) + v_steady(g))
                stage(g, q_next=True, scores=True, pv=pv(g - 1), wo=True)
                return carry

            lax.fori_loop(2, NP - 1, body, 0)
            first_layer(k_copy(NP - 1) + v_steady(NP - 2), v_last)
            stage(NP - 1 + z, q_next=False, scores=True, pv=pv(NP - 2 + z), wo=True)
            first_layer(v_last, w13_copy + sum((w2_copy(c) for c in range(len(W2_CHUNKS))), []))
            y = yp[0, 0]
            for i in range(1, (NP - 2) * NC):
                y = y + yp[i // NC, i % NC]
            yp[0, 0] = y
            stage(NP + z, q_next=False, scores=False, pv=pv_last, wo=True)
            run(mxu_wo(NP - 1))
            y = _tree_sum(yp[g, j] for g, j in
                          [(0, 0)] + [(g, j) for g in (NP - 2, NP - 1) for j in range(NC)])
            xs[...] = _round(xs[...] + _round(jnp.sum(y, axis=0, keepdims=True)))
            pl.when(it == 0)(lambda: ffn(xs[...], True))
            pl.when(it != 0)(lambda: ffn(xs[...], False))
            return carry

        dg[...] = jnp.zeros_like(dg)
        x_copy.wait()
        xs[...] = jnp.broadcast_to(xb[0].astype(F32), (8, D))
        lax.fori_loop(0, 2, layer, 0)
        o_ref[0] = xs[0:1, :].astype(o_ref.dtype)

    return kernel, nu, n_slots


@jax.jit
def pallas_interleave_layers__sliding_block_cached__glu_gated_swiglu__decode_kernel(
    A_x: jax.Array,
    A_k_cache: jax.Array,
    A_v_cache: jax.Array,
    A_wq: jax.Array,
    A_wo: jax.Array,
    B_x: jax.Array,
    B_w1: jax.Array,
    B_w3: jax.Array,
    B_w2: jax.Array,
):
    del B_x
    sk = A_k_cache.shape[2]
    win = min(4096, max(256, sk // 4))
    assert A_x.shape == (1, 1, D) and A_k_cache.shape == (1, HQ, sk, DH)
    assert win % 1024 == 0 and (sk - win) % 128 == 0
    kernel, nu, n_slots = _make_kernel(sk - win, win)

    def as_rows(c):
        return jnp.swapaxes(c, 2, 3).reshape(NP, PR, sk)

    return pl.pallas_call(
        kernel,
        out_shape=jax.ShapeDtypeStruct((1, 1, D), A_x.dtype),
        in_specs=[pl.BlockSpec(memory_space=pl.ANY)] * 8,
        scratch_shapes=[
            pltpu.VMEM((NP + 1, n_slots, PR // 2, 128), U32),
            pltpu.VMEM((NP, 4 * nu - MXU_TILES_STEADY, PR // 2, 128), U32),
            pltpu.VMEM((FC, D // 2, 128), U32),
            pltpu.VMEM((FC, D // 2, 128), U32),
            pltpu.VMEM((KC, FF // 2, 128), U32),
            pltpu.VMEM((1, 1, D), BF16),
            pltpu.VMEM((8, D), F32),
            pltpu.VMEM((8, D), F32),
            pltpu.VMEM((8, 128), F32),
            pltpu.VMEM((2, KC, 8, PR), F32),
            pltpu.VMEM((NC, 8, 128), F32),
            pltpu.VMEM((nu, 8, 128), F32),
            pltpu.VMEM((nu, 8, 128), F32),
            pltpu.VMEM((nu, 8, 128), F32),
            pltpu.VMEM((2, 4 * nu, 8, 128), F32),
            pltpu.VMEM((NC, 8, 128), F32),
            pltpu.VMEM((NC, 8, 128), F32),
            pltpu.VMEM((nu, 8, PR), F32),
            pltpu.VMEM((NC, 8, 128), F32),
            pltpu.VMEM((NP, NC, 8, D), F32),
            pltpu.SemaphoreType.DMA((NP,)),
            pltpu.SemaphoreType.DMA((NP,)),
            pltpu.SemaphoreType.DMA((4 + len(W2_CHUNKS),)),
        ],
        compiler_params=pltpu.CompilerParams(
            vmem_limit_bytes=128 * 1024 * 1024, disable_semaphore_checks=True),
        name="interleave_decode",
    )(A_x, as_rows(A_k_cache), as_rows(A_v_cache), A_wq, A_wo.reshape(NP, PR, D),
      B_w1, B_w3, B_w2)
```

```python
import jax
import jax.numpy as jnp
from jax import lax
import jax.experimental.pallas as pl
import jax.experimental.pallas.tpu as pltpu

F32, BF16, U32 = jnp.float32, jnp.bfloat16, jnp.uint32

D, HQ, DH, FF = 640, 32, 192, 1536
NP = HQ // 2
PR = 2 * DH
KC, NC, FC = D // 128, PR // 128, FF // 128
EPS = 1e-5
SCALE = DH ** -0.5

MXU_TILES_STEADY = 1
MXU_TILES_LAST = 12
MXU_TILES_FIRST = 5
MXU_TILES_PENULT = 3
W2_CHUNKS = (8, 3, 1)
MXU_SLACK = 0
ORDER = 'qvo'
ONLY_LOOP = False
FENCE_EVERY = 8
PV_BLOCK = 3
MXU_LEAD = 4


def _bf(w):
    return pltpu.bitcast(w, BF16)


def _mm(lhs, w):
    return lax.dot_general(lhs, _bf(w), (((1,), (0,)), ((), ())),
                           preferred_element_type=F32)


def _mm_t(lhs, w):
    return lax.dot_general(lhs, _bf(w), (((1,), (1,)), ((), ())),
                           preferred_element_type=F32)


def _round(x):
    return x.astype(BF16).astype(F32)


def _tree_sum(xs):
    xs = list(xs)
    while len(xs) > 1:
        xs = [xs[i] + xs[i + 1] if i + 1 < len(xs) else xs[i]
              for i in range(0, len(xs), 2)]
    return xs[0]


def _layernorm(x):
    xs = [x[:, c * 128:(c + 1) * 128] for c in range(KC)]
    c = x - jnp.sum(_tree_sum(xs), axis=-1, keepdims=True) * (1.0 / D)
    sq = _tree_sum(c[:, i * 128:(i + 1) * 128] ** 2 for i in range(KC))
    v = jnp.sum(sq, axis=-1, keepdims=True) * (1.0 / D)
    return _round(c), jnp.broadcast_to(lax.rsqrt(v + EPS), (8, 128))


def _interleave(a, na, lead, b, nb):
    ia = ib = 0
    for w in b:
        ib += w
        while (ia - lead) * nb < ib * na:
            ia += next(a, na)
    for _ in a:
        pass


def _make_kernel(s0, win):
    nt = win // 128
    nu = nt // 4
    m_steady, m_last = MXU_TILES_STEADY, MXU_TILES_LAST
    T_WO = nt
    T_WQ = T_WO + KC
    T_V = T_WQ + 2 * NC
    n_slots = max(T_V + m_steady, NC + m_last + MXU_TILES_FIRST + MXU_TILES_PENULT)

    def kernel(x_hbm, k_hbm, v_hbm, wq_hbm, wo_hbm, w1_hbm, w3_hbm, w2_hbm, o_ref,
               mb, vb, w1b, w3b, w2b, xb,
               xs, xn_s, xf, qp, ql, sa, sb, pb, pbb, rl, dg, ox, ol, yp,
               sem_k, sem_v, sem_w):
        row = lax.broadcasted_iota(jnp.int32, (8, 128), 0)
        lane = lax.broadcasted_iota(jnp.int32, (8, 128), 1)

        def group(n, src, buf, idx, sem):
            def copy(i):
                return pltpu.make_async_copy(src(i), buf.bitcast(BF16).at[idx(i)], sem)
            return n, copy

        def col(i, base=0):
            return pl.ds(pl.multiple_of(base + i * 128, 128), 128)

        def start(groups):
            for n, copy in groups:
                lax.fori_loop(0, n, lambda i, c: (copy(i).start(), c)[1], 0)

        def wait(groups):
            for n, copy in groups:
                lax.fori_loop(0, n, lambda i, c: (copy(i).wait(), c)[1], 0)

        def k_copy(g):
            return [group(nt, lambda i: k_hbm.at[g, :, col(i, s0)],
                          mb, lambda i: (g, i), sem_k.at[g])]

        def v_copy(g, m, slot, t0):
            return [group(m, lambda i: v_hbm.at[g, :, col(i, s0)],
                          mb, lambda i: (slot, t0 + i), sem_v.at[g]),
                    group(nt - m, lambda i: v_hbm.at[g, :, col(i, s0 + m * 128)],
                          vb, lambda i: (g, m - m_steady + i), sem_v.at[g])]

        x_copy = pltpu.make_async_copy(x_hbm, xb, sem_w.at[0])

        def rows(r, n=128):
            return pl.ds(pl.multiple_of(r * n, n), n)

        def tiles(src, r0, n_rows, n_cols, buf, idx, sem):
            def at(i):
                return r0 + lax.div(i, n_cols), lax.rem(i, n_cols)
            return group(n_rows * n_cols, lambda i: src.at[rows(at(i)[0]), col(at(i)[1])],
                         buf, lambda i: idx(*at(i)), sem)

        wq_copy = [
            group(NP * NC, lambda i, c=c: wq_hbm.at[pl.ds(c * 128, 128), col(i)], mb,
                  lambda i, c=c: (lax.div(i, NC), T_WQ + 2 * lax.rem(i, NC) + c // NC,
                                  pl.ds(c % NC * 128, 128)),
                  sem_w.at[1])
            for c in range(KC)]
        wo_copy = [group(NP * KC,
                         lambda i: wo_hbm.at[lax.div(i, KC), :, col(lax.rem(i, KC))], mb,
                         lambda i: (lax.div(i, KC), T_WO + lax.rem(i, KC)), sem_w.at[2])]
        w13_copy = [tiles(w, 0, KC, FC, b, lambda r, c: (c, rows(r)), sem_w.at[3])
                    for w, b in ((w1_hbm, w1b), (w3_hbm, w3b))]

        def w2_copy(c):
            return [tiles(w2_hbm, sum(W2_CHUNKS[:c]), W2_CHUNKS[c], KC, w2b,
                          lambda r, c: (c, rows(r)), sem_w.at[4 + c])]

        start(wo_copy)
        x_copy.start()
        start(wq_copy + k_copy(0))

        def mxu_scores(g):
            lhs = [ql[j] for j in range(NC)]
            for t in range(nt):
                u, r = t // 4, 2 * (t % 4)
                sa[u, r:r + 1, :] = _mm(lhs[0], mb[g, t, 0:64, :])[r:r + 1]
                yield 1
                sb[u, r:r + 2, :] = _mm(lhs[1], mb[g, t, 64:128, :])[r:r + 2]
                yield 1
                sa[u, r + 1:r + 2, :] = _mm(lhs[2], mb[g, t, 128:192, :])[r + 1:r + 2]
                yield 1

        def mxu_q(g, slot=0):
            for n in range(NC):
                for c in range(KC):
                    r0 = c % NC * 64
                    qp[slot, c, :, n * 128:(n + 1) * 128] = _mm(
                        xn_s[:, c * 128:(c + 1) * 128],
                        mb[g, T_WQ + 2 * n + c // NC, r0:r0 + 64, :])
                    yield 1

        def mxu_wo(g):
            for j in range(NC):
                o = ol[j]
                for n in range(KC):
                    yp[g, j, :, n * 128:(n + 1) * 128] = _mm(
                        o, mb[g, T_WO + n, j * 64:(j + 1) * 64, :])
                    yield 1

        def mxu_pv(m, slot, t0):
            for t in range(m):
                u, r = t // 4, 2 * (t % 4)
                p = pb[u]
                for j in range(NC):
                    ox[u, r:r + 2, j * 128:(j + 1) * 128] = _mm_t(
                        p, mb[slot, t0 + t, j * 64:(j + 1) * 64, :])[r:r + 2]
                    yield 2

        def vpu_pv(g, m):
            pending = []

            def flush():
                for d0, total in pending:
                    j, c0 = divmod(d0, 128)
                    total = jnp.broadcast_to(total, (8, 128))
                    dg[j, :, c0:c0 + 8] = total[:, c0:c0 + 8]
                pending.clear()

            for h in range(2):
                for i0 in range(0, DH // 16, PV_BLOCK):
                    acc = [None] * PV_BLOCK
                    for t in range(m, nt):
                        if i0 == 0:
                            r = 2 * (t % 4) + h
                            p = jnp.broadcast_to(pb[t // 4, r:r + 1, :], (8, 128))
                            pbb[h, t] = p
                        else:
                            p = pbb[h, t]
                        p = jnp.concatenate([p, p], axis=0)
                        for i in range(PV_BLOCK):
                            r0 = h * (DH // 2) + (i0 + i) * 8
                            v = _bf(vb[g, t - m_steady, r0:r0 + 8, :]).astype(F32) * p
                            acc[i] = v if acc[i] is None else acc[i] + v
                        if (nt - 1 - t) % FENCE_EVERY == 0:
                            for i in range(PV_BLOCK):
                                mb[NP, 0, i * 16:(i + 1) * 16, :] = pltpu.bitcast(acc[i], U32)
                        if t == nt - 1:
                            for i in range(PV_BLOCK):
                                for k in (0, 8):
                                    pending.append((
                                        h * DH + (i0 + i) * 16 + k,
                                        jnp.sum(acc[i][k:k + 8], axis=1, keepdims=True)))
                            flush()
                        yield PV_BLOCK
            flush()

        def per_head(x, op):
            x = op(x, pltpu.roll(x, 2, 0))
            return op(x, pltpu.roll(x, 4, 0))

        def q_finish(slot):
            q = _tree_sum(qp[slot, c] for c in range(KC))
            q = _round(q * jnp.concatenate([xf[...]] * NC, axis=1))
            ql[0] = q[:, :128]
            ql[1] = jnp.where((row & 1) == (lane >> 6), q[:, 128:256], 0.0)
            ql[2] = q[:, 256:]

        def softmax():
            s = [sa[u] + sb[u] for u in range(nu)]
            m = s[0]
            for x in s[1:]:
                m = jnp.maximum(m, x)
            m = jnp.max(per_head(m, jnp.maximum), axis=1, keepdims=True)
            p = [jnp.exp((x - m) * SCALE) for x in s]
            l = jnp.sum(per_head(_tree_sum(p), jnp.add), axis=1, keepdims=True)
            inv = jnp.broadcast_to(1.0 / l, (8, 128))
            inv_o = pltpu.roll(inv, 1, 0)
            even = (row & 1) == 0
            inv_a, inv_b = jnp.where(even, inv, inv_o), jnp.where(even, inv_o, inv)
            for u in range(nu):
                pb[u] = p[u]
            rl[0], rl[1], rl[2] = inv_a, jnp.where(lane < 64, inv_a, inv_b), inv_b

        def pv_finish(m):
            own = ((row & 1) == 0, (row & 1) == (lane >> 6), (row & 1) == 1)
            for j in range(NC):
                part = []
                if m < nt:
                    part.append(jnp.where((lane & 7) == row, dg[j], 0.0))
                if m >= 4:
                    part.append(jnp.where(own[j], _tree_sum(
                        ox[u, :, j * 128:(j + 1) * 128] for u in range(m // 4)), 0.0))
                if m % 4:
                    part.append(jnp.where(jnp.logical_and(own[j], row < 2 * (m % 4)),
                                          ox[m // 4, :, j * 128:(j + 1) * 128], 0.0))
                ol[j] = _round(_tree_sum(part) * rl[j])

        def stage(g, *, q_next, scores, pv, wo):
            mxu, vpu, n_vpu = [], iter(()), 0
            if ONLY_LOOP and not (q_next and wo):
                return
            if pv is not None and pv[0] < nt:
                vpu, n_vpu = vpu_pv(g - 1, pv[0]), (nt - pv[0]) * PR // 16
            if scores:
                mxu.append((mxu_scores(g), NC * nt))
            if q_next:
                mxu.append((mxu_q(g + 1), NC * KC))
            if pv is not None:
                mxu.append((mxu_pv(*pv), 2 * NC * pv[0]))
            if wo:
                mxu.append((mxu_wo(g - 2), NC * KC))
            _interleave((w for s, _ in mxu for w in s), sum(n for _, n in mxu) + MXU_SLACK,
                        MXU_LEAD, vpu, n_vpu)
            if pv is not None:
                pv_finish(pv[0])
            if scores:
                softmax()
            if q_next:
                q_finish(0)

        def run(stream):
            for _ in stream:
                pass

        def ffn(x, loading):
            xn, factor = _layernorm(x)
            if loading:
                wait(w13_copy)
            h = []
            for f in range(FC):
                gate, up = (
                    _round(factor * _tree_sum(
                        _mm(xn[:, c * 128:(c + 1) * 128], w[f, c * 64:(c + 1) * 64, :])
                        for c in range(KC)))
                    for w in (w1b, w3b))
                h.append(_round(_round(gate * jax.nn.sigmoid(gate)) * up))
            y = [None] * KC
            for c, size in enumerate(W2_CHUNKS):
                if loading:
                    wait(w2_copy(c))
                for f in range(sum(W2_CHUNKS[:c]), sum(W2_CHUNKS[:c + 1])):
                    for n in range(KC):
                        r = _mm(h[f], w2b[n, f * 64:(f + 1) * 64, :])
                        y[n] = r if y[n] is None else y[n] + r
            xs[...] = _round(x + _round(jnp.concatenate(y, axis=1)))

        def layer(it, carry):
            z = it >> 1

            def first_layer(await_, start_=()):
                @pl.when(it == 0)
                def _():
                    start(start_)
                    wait(await_)

            def pv(g):
                return m_steady, g, T_V

            def v_steady(g):
                return v_copy(g, *pv(g))

            pv_last = (m_last, NP + z, NC)
            pv_first = (MXU_TILES_FIRST, NP + z, NC + m_last)
            pv_penult = (MXU_TILES_PENULT, NP + z, NC + m_last + MXU_TILES_FIRST)
            v_last = v_copy(NP - 1, *pv_last)

            v_first, v_penult = v_copy(0, *pv_first), v_copy(NP - 2, *pv_penult)

            first_layer(wo_copy + wq_copy + k_copy(0), k_copy(1) + v_first)
            xn_s[...], xf[...] = _layernorm(xs[...])
            run(mxu_q(0, 0))
            run(mxu_q(1, 1))
            q_finish(0)
            stage(z, q_next=False, scores=True, pv=None, wo=False)
            run(mxu_q(2, 0))
            q_finish(1)
            first_layer(k_copy(1) + v_first, k_copy(2) + v_steady(1))
            stage(1 + z, q_next=False, scores=True, pv=pv_first, wo=False)
            q_finish(0)

            def body(g, carry):
                @pl.when(it == 0)
                def _():
                    start(k_copy(g + 1))
                    pl.when(g < NP - 2)(lambda: start(v_steady(g)))
                    pl.when(g == NP - 2)(lambda: start(v_penult))
                    wait(k_copy(g) + v_steady(g - 1))
                stage(g, q_next=True, scores=True, pv=pv(g - 1), wo=True)
                return carry

            lax.fori_loop(2, NP - 1, body, 0)
            first_layer(k_copy(NP - 1) + v_penult, v_last)
            stage(NP - 1 + z, q_next=False, scores=True, pv=pv_penult, wo=True)
            first_layer(v_last, w13_copy + sum((w2_copy(c) for c in range(len(W2_CHUNKS))), []))
            y = yp[0, 0]
            for i in range(1, (NP - 2) * NC):
                y = y + yp[i // NC, i % NC]
            yp[0, 0] = y
            stage(NP + z, q_next=False, scores=False, pv=pv_last, wo=True)
            run(mxu_wo(NP - 1))
            y = _tree_sum(yp[g, j] for g, j in
                          [(0, 0)] + [(g, j) for g in (NP - 2, NP - 1) for j in range(NC)])
            xs[...] = _round(xs[...] + _round(jnp.sum(y, axis=0, keepdims=True)))
            pl.when(it == 0)(lambda: ffn(xs[...], True))
            pl.when(it != 0)(lambda: ffn(xs[...], False))
            return carry

        dg[...] = jnp.zeros_like(dg)
        x_copy.wait()
        xs[...] = jnp.broadcast_to(xb[0].astype(F32), (8, D))
        lax.fori_loop(0, 2, layer, 0)
        o_ref[0] = xs[0:1, :].astype(o_ref.dtype)

    return kernel, nu, n_slots


@jax.jit
def pallas_interleave_layers__sliding_block_cached__glu_gated_swiglu__decode_kernel(
    A_x: jax.Array,
    A_k_cache: jax.Array,
    A_v_cache: jax.Array,
    A_wq: jax.Array,
    A_wo: jax.Array,
    B_x: jax.Array,
    B_w1: jax.Array,
    B_w3: jax.Array,
    B_w2: jax.Array,
):
    del B_x
    sk = A_k_cache.shape[2]
    win = min(4096, max(256, sk // 4))
    assert A_x.shape == (1, 1, D) and A_k_cache.shape == (1, HQ, sk, DH)
    assert win % 1024 == 0 and (sk - win) % 128 == 0
    kernel, nu, n_slots = _make_kernel(sk - win, win)

    def as_rows(c):
        return jnp.swapaxes(c, 2, 3).reshape(NP, PR, sk)

    return pl.pallas_call(
        kernel,
        out_shape=jax.ShapeDtypeStruct((1, 1, D), A_x.dtype),
        in_specs=[pl.BlockSpec(memory_space=pl.ANY)] * 8,
        scratch_shapes=[
            pltpu.VMEM((NP + 1, n_slots, PR // 2, 128), U32),
            pltpu.VMEM((NP, 4 * nu - MXU_TILES_STEADY, PR // 2, 128), U32),
            pltpu.VMEM((FC, D // 2, 128), U32),
            pltpu.VMEM((FC, D // 2, 128), U32),
            pltpu.VMEM((KC, FF // 2, 128), U32),
            pltpu.VMEM((1, 1, D), BF16),
            pltpu.VMEM((8, D), F32),
            pltpu.VMEM((8, D), F32),
            pltpu.VMEM((8, 128), F32),
            pltpu.VMEM((2, KC, 8, PR), F32),
            pltpu.VMEM((NC, 8, 128), F32),
            pltpu.VMEM((nu, 8, 128), F32),
            pltpu.VMEM((nu, 8, 128), F32),
            pltpu.VMEM((nu, 8, 128), F32),
            pltpu.VMEM((2, 4 * nu, 8, 128), F32),
            pltpu.VMEM((NC, 8, 128), F32),
            pltpu.VMEM((NC, 8, 128), F32),
            pltpu.VMEM((nu, 8, PR), F32),
            pltpu.VMEM((NC, 8, 128), F32),
            pltpu.VMEM((NP, NC, 8, D), F32),
            pltpu.SemaphoreType.DMA((NP,)),
            pltpu.SemaphoreType.DMA((NP,)),
            pltpu.SemaphoreType.DMA((4 + len(W2_CHUNKS),)),
        ],
        compiler_params=pltpu.CompilerParams(
            vmem_limit_bytes=128 * 1024 * 1024, disable_semaphore_checks=True),
        name="interleave_decode",
    )(A_x, as_rows(A_k_cache), as_rows(A_v_cache), A_wq, A_wo.reshape(NP, PR, D),
      B_w1, B_w3, B_w2)
```

```python
import jax
import jax.numpy as jnp
from jax import lax
import jax.experimental.pallas as pl
import jax.experimental.pallas.tpu as pltpu

F32, BF16, U32 = jnp.float32, jnp.bfloat16, jnp.uint32

D, HQ, DH, FF = 640, 32, 192, 1536
NP = HQ // 2
PR = 2 * DH
KC, NC, FC = D // 128, PR // 128, FF // 128
EPS = 1e-5
SCALE = DH ** -0.5

MXU_TILES_STEADY = 2
MXU_TILES_LAST = 16
MXU_TILES_FIRST = 8
MXU_TILES_PENULT = 4
W2_CHUNKS = (8, 3, 1)
MXU_SLACK = 0
ONLY_LOOP = False
FENCE_EVERY = 8
PV_BLOCK = 3
MXU_LEAD = 4


def _bf(w):
    return pltpu.bitcast(w, BF16)


def _mm(lhs, w):
    return lax.dot_general(lhs, _bf(w), (((1,), (0,)), ((), ())),
                           preferred_element_type=F32)


def _round(x):
    return x.astype(BF16).astype(F32)


def _tree_sum(xs):
    xs = list(xs)
    while len(xs) > 1:
        xs = [xs[i] + xs[i + 1] if i + 1 < len(xs) else xs[i]
              for i in range(0, len(xs), 2)]
    return xs[0]


def _layernorm(x):
    xs = [x[:, c * 128:(c + 1) * 128] for c in range(KC)]
    c = x - jnp.sum(_tree_sum(xs), axis=-1, keepdims=True) * (1.0 / D)
    sq = _tree_sum(c[:, i * 128:(i + 1) * 128] ** 2 for i in range(KC))
    v = jnp.sum(sq, axis=-1, keepdims=True) * (1.0 / D)
    return _round(c), jnp.broadcast_to(lax.rsqrt(v + EPS), (8, 128))


def _interleave(a, na, lead, b, nb):
    ia = ib = 0
    for w in b:
        ib += w
        while (ia - lead) * nb < ib * na:
            ia += next(a, na)
    for _ in a:
        pass


def _make_kernel(s0, win):
    nt = win // 128
    nu = nt // 4
    m_steady, m_last = MXU_TILES_STEADY, MXU_TILES_LAST
    T_WO = nt
    T_WQ = T_WO + KC
    T_V = T_WQ + 2 * NC
    n_slots = max(T_V + m_steady, NC + m_last + MXU_TILES_FIRST + MXU_TILES_PENULT)

    def kernel(x_hbm, k_hbm, v_hbm, wq_hbm, wo_hbm, w1_hbm, w3_hbm, w2_hbm, o_ref,
               mb, vb, w1b, w3b, w2b, xb,
               xs, xn_s, xf, qp, ql, sa, sb, pb, pbb, rl, dg, ox, ol, yp,
               sem_k, sem_v, sem_w):
        row = lax.broadcasted_iota(jnp.int32, (8, 128), 0)
        lane = lax.broadcasted_iota(jnp.int32, (8, 128), 1)

        def group(n, src, buf, idx, sem):
            def copy(i):
                return pltpu.make_async_copy(src(i), buf.bitcast(BF16).at[idx(i)], sem)
            return n, copy

        def col(i, base=0):
            return pl.ds(pl.multiple_of(base + i * 128, 128), 128)

        def start(groups):
            for n, copy in groups:
                lax.fori_loop(0, n, lambda i, c: (copy(i).start(), c)[1], 0)

        def wait(groups):
            for n, copy in groups:
                lax.fori_loop(0, n, lambda i, c: (copy(i).wait(), c)[1], 0)

        def k_copy(g):
            return [group(nt, lambda i: k_hbm.at[g, :, col(i, s0)],
                          mb, lambda i: (g, i), sem_k.at[g])]

        def v_head(g, m, slot, t0, sem):
            return [group(m, lambda i: v_hbm.at[g, :, col(i, s0)],
                          mb, lambda i: (slot, t0 + i), sem)]

        def v_rest(g, m):
            return [group(nt - m, lambda i: v_hbm.at[g, :, col(i, s0 + m * 128)],
                          vb, lambda i: (g, m - m_steady + i), sem_v.at[g])]

        x_copy = pltpu.make_async_copy(x_hbm, xb, sem_w.at[0])

        def rows(r, n=128):
            return pl.ds(pl.multiple_of(r * n, n), n)

        def tiles(src, r0, n_rows, n_cols, buf, idx, sem):
            def at(i):
                return r0 + lax.div(i, n_cols), lax.rem(i, n_cols)
            return group(n_rows * n_cols, lambda i: src.at[rows(at(i)[0]), col(at(i)[1])],
                         buf, lambda i: idx(*at(i)), sem)

        wq_copy = [
            group(NP * NC, lambda i, c=c: wq_hbm.at[pl.ds(c * 128, 128), col(i)], mb,
                  lambda i, c=c: (lax.div(i, NC), T_WQ + 2 * lax.rem(i, NC) + c // NC,
                                  pl.ds(c % NC * 128, 128)),
                  sem_w.at[1])
            for c in range(KC)]
        wo_copy = [group(NP * KC,
                         lambda i: wo_hbm.at[lax.div(i, KC), :, col(lax.rem(i, KC))], mb,
                         lambda i: (lax.div(i, KC), T_WO + lax.rem(i, KC)), sem_w.at[2])]
        w13_copy = [tiles(w, 0, KC, FC, b, lambda r, c: (c, rows(r)), sem_w.at[3])
                    for w, b in ((w1_hbm, w1b), (w3_hbm, w3b))]

        def w2_copy(c):
            return [tiles(w2_hbm, sum(W2_CHUNKS[:c]), W2_CHUNKS[c], KC, w2b,
                          lambda r, c: (c, rows(r)), sem_w.at[5 + c])]

        start(wo_copy)
        x_copy.start()
        start(wq_copy + k_copy(0))

        def mxu_scores(g):
            lhs = [ql[j] for j in range(NC)]
            for t in range(nt):
                u, r = t // 4, 2 * (t % 4)
                sa[u, r:r + 1, :] = _mm(lhs[0], mb[g, t, 0:64, :])[r:r + 1]
                yield 1
                sb[u, r:r + 2, :] = _mm(lhs[1], mb[g, t, 64:128, :])[r:r + 2]
                yield 1
                sa[u, r + 1:r + 2, :] = _mm(lhs[2], mb[g, t, 128:192, :])[r + 1:r + 2]
                yield 1

        def mxu_q(g, slot=0):
            for n in range(NC):
                for c in range(KC):
                    r0 = c % NC * 64
                    qp[slot, c, :, n * 128:(n + 1) * 128] = _mm(
                        xn_s[:, c * 128:(c + 1) * 128],
                        mb[g, T_WQ + 2 * n + c // NC, r0:r0 + 64, :])
                    yield 1

        def mxu_wo(g):
            for j in range(NC):
                o = ol[j]
                for n in range(KC):
                    yp[g, j, :, n * 128:(n + 1) * 128] = _mm(
                        o, mb[g, T_WO + n, j * 64:(j + 1) * 64, :])
                    yield 1

        def mxu_pv(m, slot, t0):
            for t in range(m):
                u, r = t // 4, 2 * (t % 4)
                p = _round(pb[u])
                for j in range(NC):
                    ox[u, r:r + 2, j * 128:(j + 1) * 128] = _mm(
                        p, mb[slot, t0 + t, j * 64:(j + 1) * 64, :])[r:r + 2]
                    yield 1

        def vpu_pv(g, m):
            pending = []

            def flush():
                for d0, total in pending:
                    j, c0 = divmod(d0, 128)
                    total = jnp.broadcast_to(total, (8, 128))
                    dg[j, :, c0:c0 + 8] = total[:, c0:c0 + 8]
                pending.clear()

            for h in range(2):
                for i0 in range(0, DH // 16, PV_BLOCK):
                    acc = [None] * PV_BLOCK
                    for t in range(m, nt):
                        if i0 == 0:
                            r = 2 * (t % 4) + h
                            p = jnp.broadcast_to(pb[t // 4, r:r + 1, :], (8, 128))
                            pbb[h, t] = p
                        else:
                            p = pbb[h, t]
                        p = jnp.concatenate([p, p], axis=0)
                        for i in range(PV_BLOCK):
                            r0 = h * (DH // 2) + (i0 + i) * 8
                            v = _bf(vb[g, t - m_steady, r0:r0 + 8, :]).astype(F32) * p
                            acc[i] = v if acc[i] is None else acc[i] + v
                        if (nt - 1 - t) % FENCE_EVERY == 0:
                            for i in range(PV_BLOCK):
                                mb[NP, 0, i * 16:(i + 1) * 16, :] = pltpu.bitcast(acc[i], U32)
                        if t == nt - 1:
                            for i in range(PV_BLOCK):
                                for k in (0, 8):
                                    pending.append((
                                        h * DH + (i0 + i) * 16 + k,
                                        jnp.sum(acc[i][k:k + 8], axis=1, keepdims=True)))
                            flush()
                        yield PV_BLOCK
            flush()

        def per_head(x, op):
            x = op(x, pltpu.roll(x, 2, 0))
            return op(x, pltpu.roll(x, 4, 0))

        def q_finish(slot):
            q = _tree_sum(qp[slot, c] for c in range(KC))
            q = _round(q * jnp.concatenate([xf[...]] * NC, axis=1))
            ql[0] = q[:, :128]
            ql[1] = jnp.where((row & 1) == (lane >> 6), q[:, 128:256], 0.0)
            ql[2] = q[:, 256:]

        def softmax():
            s = [sa[u] + sb[u] for u in range(nu)]
            m = s[0]
            for x in s[1:]:
                m = jnp.maximum(m, x)
            m = jnp.max(per_head(m, jnp.maximum), axis=1, keepdims=True)
            p = [jnp.exp((x - m) * SCALE) for x in s]
            l = jnp.sum(per_head(_tree_sum(p), jnp.add), axis=1, keepdims=True)
            inv = jnp.broadcast_to(1.0 / l, (8, 128))
            inv_o = pltpu.roll(inv, 1, 0)
            even = (row & 1) == 0
            inv_a, inv_b = jnp.where(even, inv, inv_o), jnp.where(even, inv_o, inv)
            for u in range(nu):
                pb[u] = p[u]
            rl[0], rl[1], rl[2] = inv_a, jnp.where(lane < 64, inv_a, inv_b), inv_b

        def pv_finish(m):
            own = ((row & 1) == 0, (row & 1) == (lane >> 6), (row & 1) == 1)
            for j in range(NC):
                part = []
                if m < nt:
                    part.append(jnp.where((lane & 7) == row, dg[j], 0.0))
                if m >= 4:
                    part.append(jnp.where(own[j], _tree_sum(
                        ox[u, :, j * 128:(j + 1) * 128] for u in range(m // 4)), 0.0))
                if m % 4:
                    part.append(jnp.where(jnp.logical_and(own[j], row < 2 * (m % 4)),
                                          ox[m // 4, :, j * 128:(j + 1) * 128], 0.0))
                ol[j] = _round(_tree_sum(part) * rl[j])

        def stage(g, *, q_next, scores, pv, wo):
            mxu, vpu, n_vpu = [], iter(()), 0
            if ONLY_LOOP and not (q_next and wo):
                return
            if pv is not None and pv[0] < nt:
                vpu, n_vpu = vpu_pv(g - 1, pv[0]), (nt - pv[0]) * PR // 16
            if scores:
                mxu.append((mxu_scores(g), NC * nt))
            if q_next:
                mxu.append((mxu_q(g + 1), NC * KC))
            if pv is not None:
                mxu.append((mxu_pv(*pv), NC * pv[0]))
            if wo:
                mxu.append((mxu_wo(g - 2), NC * KC))
            _interleave((w for s, _ in mxu for w in s), sum(n for _, n in mxu) + MXU_SLACK,
                        MXU_LEAD, vpu, n_vpu)
            if pv is not None:
                pv_finish(pv[0])
            if scores:
                softmax()
            if q_next:
                q_finish(0)

        def run(stream):
            for _ in stream:
                pass

        def ffn(x, loading):
            xn, factor = _layernorm(x)
            if loading:
                wait(w13_copy)
            h = []
            for f in range(FC):
                gate, up = (
                    _round(factor * _tree_sum(
                        _mm(xn[:, c * 128:(c + 1) * 128], w[f, c * 64:(c + 1) * 64, :])
                        for c in range(KC)))
                    for w in (w1b, w3b))
                h.append(_round(_round(gate * jax.nn.sigmoid(gate)) * up))
            y = [None] * KC
            for c, size in enumerate(W2_CHUNKS):
                if loading:
                    wait(w2_copy(c))
                for f in range(sum(W2_CHUNKS[:c]), sum(W2_CHUNKS[:c + 1])):
                    for n in range(KC):
                        r = _mm(h[f], w2b[n, f * 64:(f + 1) * 64, :])
                        y[n] = r if y[n] is None else y[n] + r
            xs[...] = _round(x + _round(jnp.concatenate(y, axis=1)))

        def transpose(m, slot, t0):
            def one(i, carry):
                for j in range(NC):
                    at = (slot, t0 + i, slice(j * 64, (j + 1) * 64))
                    mb[at] = pltpu.bitcast(_bf(mb[at]).astype(F32).T.astype(BF16), U32)
                return carry
            lax.fori_loop(0, m, one, 0)

        def layer(it, carry):
            z = it >> 1

            def first_layer(await_, start_, *fresh):
                @pl.when(it == 0)
                def _():
                    start(start_)
                    wait(await_)
                    for tiles_ in fresh:
                        transpose(*tiles_)

            def pv(g):
                return m_steady, g, T_V

            def v_steady(g):
                return v_head(g, *pv(g), sem_v.at[g]) + v_rest(g, m_steady)

            pv_last = (m_last, NP + z, NC)
            pv_first = (MXU_TILES_FIRST, NP + z, NC + m_last)
            pv_penult = (MXU_TILES_PENULT, NP + z, NC + m_last + MXU_TILES_FIRST)
            v_last = v_rest(NP - 1, m_last)

            v_first, v_penult = v_rest(0, pv_first[0]), v_rest(NP - 2, pv_penult[0])
            v_spare = sum((v_head(g, *at, sem_w.at[4]) for g, at in
                           ((NP - 1, pv_last), (0, pv_first), (NP - 2, pv_penult))), [])

            first_layer(wo_copy + wq_copy + k_copy(0), v_spare + k_copy(1) + v_first)
            xn_s[...], xf[...] = _layernorm(xs[...])
            run(mxu_q(0, 0))
            run(mxu_q(1, 1))
            q_finish(0)
            stage(z, q_next=False, scores=True, pv=None, wo=False)
            run(mxu_q(2, 0))
            q_finish(1)
            first_layer(v_spare + k_copy(1) + v_first, k_copy(2) + v_steady(1),
                        (m_last + pv_first[0] + pv_penult[0], NP, NC))
            stage(1 + z, q_next=False, scores=True, pv=pv_first, wo=False)
            q_finish(0)

            def body(g, carry):
                @pl.when(it == 0)
                def _():
                    start(k_copy(g + 1))
                    pl.when(g < NP - 2)(lambda: start(v_steady(g)))
                    pl.when(g == NP - 2)(lambda: start(v_penult))
                    wait(k_copy(g) + v_steady(g - 1))
                    transpose(*pv(g - 1))
                stage(g, q_next=True, scores=True, pv=pv(g - 1), wo=True)
                return carry

            lax.fori_loop(2, NP - 1, body, 0)
            first_layer(k_copy(NP - 1) + v_penult, v_last)
            stage(NP - 1 + z, q_next=False, scores=True, pv=pv_penult, wo=True)
            first_layer(v_last, w13_copy + sum((w2_copy(c) for c in range(len(W2_CHUNKS))), []))
            y = yp[0, 0]
            for i in range(1, (NP - 2) * NC):
                y = y + yp[i // NC, i % NC]
            yp[0, 0] = y
            stage(NP + z, q_next=False, scores=False, pv=pv_last, wo=True)
            run(mxu_wo(NP - 1))
            y = _tree_sum(yp[g, j] for g, j in
                          [(0, 0)] + [(g, j) for g in (NP - 2, NP - 1) for j in range(NC)])
            xs[...] = _round(xs[...] + _round(jnp.sum(y, axis=0, keepdims=True)))
            pl.when(it == 0)(lambda: ffn(xs[...], True))
            pl.when(it != 0)(lambda: ffn(xs[...], False))
            return carry

        dg[...] = jnp.zeros_like(dg)
        x_copy.wait()
        xs[...] = jnp.broadcast_to(xb[0].astype(F32), (8, D))
        lax.fori_loop(0, 2, layer, 0)
        o_ref[0] = xs[0:1, :].astype(o_ref.dtype)

    return kernel, nu, n_slots


@jax.jit
def pallas_interleave_layers__sliding_block_cached__glu_gated_swiglu__decode_kernel(
    A_x: jax.Array,
    A_k_cache: jax.Array,
    A_v_cache: jax.Array,
    A_wq: jax.Array,
    A_wo: jax.Array,
    B_x: jax.Array,
    B_w1: jax.Array,
    B_w3: jax.Array,
    B_w2: jax.Array,
):
    del B_x
    sk = A_k_cache.shape[2]
    win = min(4096, max(256, sk // 4))
    assert A_x.shape == (1, 1, D) and A_k_cache.shape == (1, HQ, sk, DH)
    assert win % 1024 == 0 and (sk - win) % 128 == 0
    kernel, nu, n_slots = _make_kernel(sk - win, win)

    def as_rows(c):
        return jnp.swapaxes(c, 2, 3).reshape(NP, PR, sk)

    return pl.pallas_call(
        kernel,
        out_shape=jax.ShapeDtypeStruct((1, 1, D), A_x.dtype),
        in_specs=[pl.BlockSpec(memory_space=pl.ANY)] * 8,
        scratch_shapes=[
            pltpu.VMEM((NP + 1, n_slots, PR // 2, 128), U32),
            pltpu.VMEM((NP, 4 * nu - MXU_TILES_STEADY, PR // 2, 128), U32),
            pltpu.VMEM((FC, D // 2, 128), U32),
            pltpu.VMEM((FC, D // 2, 128), U32),
            pltpu.VMEM((KC, FF // 2, 128), U32),
            pltpu.VMEM((1, 1, D), BF16),
            pltpu.VMEM((8, D), F32),
            pltpu.VMEM((8, D), F32),
            pltpu.VMEM((8, 128), F32),
            pltpu.VMEM((2, KC, 8, PR), F32),
            pltpu.VMEM((NC, 8, 128), F32),
            pltpu.VMEM((nu, 8, 128), F32),
            pltpu.VMEM((nu, 8, 128), F32),
            pltpu.VMEM((nu, 8, 128), F32),
            pltpu.VMEM((2, 4 * nu, 8, 128), F32),
            pltpu.VMEM((NC, 8, 128), F32),
            pltpu.VMEM((NC, 8, 128), F32),
            pltpu.VMEM((nu, 8, PR), F32),
            pltpu.VMEM((NC, 8, 128), F32),
            pltpu.VMEM((NP, NC, 8, D), F32),
            pltpu.SemaphoreType.DMA((NP,)),
            pltpu.SemaphoreType.DMA((NP,)),
            pltpu.SemaphoreType.DMA((5 + len(W2_CHUNKS),)),
        ],
        compiler_params=pltpu.CompilerParams(
            vmem_limit_bytes=128 * 1024 * 1024, disable_semaphore_checks=True),
        name="interleave_decode",
    )(A_x, as_rows(A_k_cache), as_rows(A_v_cache), A_wq, A_wo.reshape(NP, PR, D),
      B_w1, B_w3, B_w2)
```

```python
import jax
import jax.numpy as jnp
from jax import lax
import jax.experimental.pallas as pl
import jax.experimental.pallas.tpu as pltpu

F32, BF16, U32 = jnp.float32, jnp.bfloat16, jnp.uint32

D, HQ, DH, FF = 640, 32, 192, 1536
NP = HQ // 2
PR = 2 * DH
KC, NC, FC = D // 128, PR // 128, FF // 128
EPS = 1e-5
SCALE = DH ** -0.5

M_STEADY = 4
M_FIRST = 8
M_PENULT = 8
M_LAST = 16
W2_CHUNKS = (8, 3, 1)
PV_BLOCK = 3
PACE_EVERY = 7


def _bf(w):
    return pltpu.bitcast(w, BF16)


def _mm(lhs, w):
    return lax.dot_general(lhs, _bf(w), (((1,), (0,)), ((), ())),
                           preferred_element_type=F32)


def _round(x):
    return x.astype(BF16).astype(F32)


def _tree_sum(xs):
    xs = list(xs)
    while len(xs) > 1:
        xs = [xs[i] + xs[i + 1] if i + 1 < len(xs) else xs[i]
              for i in range(0, len(xs), 2)]
    return xs[0]


def _layernorm(x):
    xs = [x[:, c * 128:(c + 1) * 128] for c in range(KC)]
    c = x - jnp.sum(_tree_sum(xs), axis=-1, keepdims=True) * (1.0 / D)
    sq = _tree_sum(c[:, i * 128:(i + 1) * 128] ** 2 for i in range(KC))
    v = jnp.sum(sq, axis=-1, keepdims=True) * (1.0 / D)
    return _round(c), jnp.broadcast_to(lax.rsqrt(v + EPS), (8, 128))


def _interleave(a, na, b, nb):
    ia = ib = 0
    for w in b:
        ib += w
        while ia * nb < ib * na:
            ia += next(a, na)
    for _ in a:
        pass


def _make_kernel(s0, win):
    nt = win // 128
    nu = nt // 4
    T_WO = nt
    T_WQ = T_WO + KC
    T_V = T_WQ + 2 * NC
    n_slots = max(T_V + M_STEADY, NC + M_LAST + M_FIRST + M_PENULT)

    def kernel(x_hbm, k_hbm, v_hbm, wq_hbm, wo_hbm, w1_hbm, w3_hbm, w2_hbm, o_ref,
               mb, vb, w1b, w3b, w2b, xb,
               xs, xn_s, xf, qp, ql, sa, sb, pb, pbb, rl, dg, ox, ol, yp,
               sem_k, sem_v, sem_w):
        row = lax.broadcasted_iota(jnp.int32, (8, 128), 0)
        lane = lax.broadcasted_iota(jnp.int32, (8, 128), 1)

        def group(n, src, buf, idx, sem):
            def copy(i):
                return pltpu.make_async_copy(src(i), buf.bitcast(BF16).at[idx(i)], sem)
            return n, copy

        def col(i, base=0):
            return pl.ds(pl.multiple_of(base + i * 128, 128), 128)

        def start(groups):
            for n, copy in groups:
                lax.fori_loop(0, n, lambda i, c: (copy(i).start(), c)[1], 0)

        def wait(groups):
            for n, copy in groups:
                lax.fori_loop(0, n, lambda i, c: (copy(i).wait(), c)[1], 0)

        def k_copy(g):
            return [group(nt, lambda i: k_hbm.at[g, :, col(i, s0)],
                          mb, lambda i: (g, i), sem_k.at[g])]

        def v_head(g, m, slot, t0, sem):
            return [group(m, lambda i: v_hbm.at[g, :, col(i, s0)],
                          mb, lambda i: (slot, t0 + i), sem)]

        def v_rest(g, m):
            return [group(nt - m, lambda i: v_hbm.at[g, :, col(i, s0 + m * 128)],
                          vb, lambda i: (g, m - M_STEADY + i), sem_v.at[g])]

        x_copy = pltpu.make_async_copy(x_hbm, xb, sem_w.at[0])

        def rows(r, n=128):
            return pl.ds(pl.multiple_of(r * n, n), n)

        def tiles(src, r0, n_rows, n_cols, buf, idx, sem):
            def at(i):
                return r0 + lax.div(i, n_cols), lax.rem(i, n_cols)
            return group(n_rows * n_cols, lambda i: src.at[rows(at(i)[0]), col(at(i)[1])],
                         buf, lambda i: idx(*at(i)), sem)

        wq_copy = [
            group(NP * NC, lambda i, c=c: wq_hbm.at[pl.ds(c * 128, 128), col(i)], mb,
                  lambda i, c=c: (lax.div(i, NC), T_WQ + 2 * lax.rem(i, NC) + c // NC,
                                  pl.ds(c % NC * 128, 128)),
                  sem_w.at[1])
            for c in range(KC)]
        wo_copy = [group(NP * KC,
                         lambda i: wo_hbm.at[lax.div(i, KC), :, col(lax.rem(i, KC))], mb,
                         lambda i: (lax.div(i, KC), T_WO + lax.rem(i, KC)), sem_w.at[2])]
        w13_copy = [tiles(w, 0, KC, FC, b, lambda r, c: (c, rows(r)), sem_w.at[3])
                    for w, b in ((w1_hbm, w1b), (w3_hbm, w3b))]

        def w2_copy(c):
            return [tiles(w2_hbm, sum(W2_CHUNKS[:c]), W2_CHUNKS[c], KC, w2b,
                          lambda r, c: (c, rows(r)), sem_w.at[5 + c])]

        start(wo_copy)
        x_copy.start()
        start(wq_copy + k_copy(0))

        def mxu_scores(g):
            lhs = [ql[j] for j in range(NC)]
            for t in range(nt):
                u, r = t // 4, 2 * (t % 4)
                sa[u, r:r + 1, :] = _mm(lhs[0], mb[g, t, 0:64, :])[r:r + 1]
                yield 1
                sb[u, r:r + 2, :] = _mm(lhs[1], mb[g, t, 64:128, :])[r:r + 2]
                yield 1
                sa[u, r + 1:r + 2, :] = _mm(lhs[2], mb[g, t, 128:192, :])[r + 1:r + 2]
                yield 1

        def mxu_q(g, slot):
            for n in range(NC):
                for c in range(KC):
                    r0 = c % NC * 64
                    qp[slot, c, :, n * 128:(n + 1) * 128] = _mm(
                        xn_s[:, c * 128:(c + 1) * 128],
                        mb[g, T_WQ + 2 * n + c // NC, r0:r0 + 64, :])
                    yield 1

        def mxu_wo(g):
            for j in range(NC):
                o = ol[j]
                for n in range(KC):
                    yp[g, j, :, n * 128:(n + 1) * 128] = _mm(
                        o, mb[g, T_WO + n, j * 64:(j + 1) * 64, :])
                    yield 1

        def mxu_pv(m, slot, t0):
            for t in range(m):
                u, r = t // 4, 2 * (t % 4)
                p = _round(pb[u])
                for j in range(NC):
                    ox[u, r:r + 2, j * 128:(j + 1) * 128] = _mm(
                        p, mb[slot, t0 + t, j * 64:(j + 1) * 64, :])[r:r + 2]
                    yield 1

        def vpu_pv(g, m):
            for h in range(2):
                for i0 in range(0, DH // 16, PV_BLOCK):
                    acc = [None] * PV_BLOCK
                    for t in range(m, nt):
                        if i0 == 0:
                            r = 2 * (t % 4) + h
                            p = jnp.broadcast_to(pb[t // 4, r:r + 1, :], (8, 128))
                            pbb[h, t] = p
                        else:
                            p = pbb[h, t]
                        p = jnp.concatenate([p, p], axis=0)
                        for i in range(PV_BLOCK):
                            r0 = h * (DH // 2) + (i0 + i) * 8
                            v = _bf(vb[g, t - M_STEADY, r0:r0 + 8, :]).astype(F32) * p
                            acc[i] = v if acc[i] is None else acc[i] + v
                        if (nt - 1 - t) % PACE_EVERY == 0:
                            for i in range(PV_BLOCK):
                                mb[NP, 0, i * 16:(i + 1) * 16, :] = pltpu.bitcast(acc[i], U32)
                        if t == nt - 1:
                            sums = [jnp.sum(x[k:k + 8], axis=1, keepdims=True)
                                    for x in acc for k in (0, 8)]
                            for i, x in enumerate(sums):
                                j, c0 = divmod(h * DH + i0 * 16 + i * 8, 128)
                                x = jnp.broadcast_to(x, (8, 128))
                                dg[j, :, c0:c0 + 8] = x[:, c0:c0 + 8]
                        yield PV_BLOCK

        def per_head(x, op):
            x = op(x, pltpu.roll(x, 2, 0))
            return op(x, pltpu.roll(x, 4, 0))

        def q_finish(slot):
            q = _tree_sum(qp[slot, c] for c in range(KC))
            q = _round(q * jnp.concatenate([xf[...]] * NC, axis=1))
            ql[0] = q[:, :128]
            ql[1] = jnp.where((row & 1) == (lane >> 6), q[:, 128:256], 0.0)
            ql[2] = q[:, 256:]

        def softmax():
            s = [sa[u] + sb[u] for u in range(nu)]
            m = s[0]
            for x in s[1:]:
                m = jnp.maximum(m, x)
            m = jnp.max(per_head(m, jnp.maximum), axis=1, keepdims=True)
            p = [jnp.exp((x - m) * SCALE) for x in s]
            l = jnp.sum(per_head(_tree_sum(p), jnp.add), axis=1, keepdims=True)
            inv = jnp.broadcast_to(1.0 / l, (8, 128))
            inv_o = pltpu.roll(inv, 1, 0)
            even = (row & 1) == 0
            inv_a, inv_b = jnp.where(even, inv, inv_o), jnp.where(even, inv_o, inv)
            for u in range(nu):
                pb[u] = p[u]
            rl[0], rl[1], rl[2] = inv_a, jnp.where(lane < 64, inv_a, inv_b), inv_b

        def pv_finish(m):
            own = ((row & 1) == 0, (row & 1) == (lane >> 6), (row & 1) == 1)
            for j in range(NC):
                o = jnp.where((lane & 7) == row, dg[j], 0.0) + jnp.where(own[j], _tree_sum(
                    ox[u, :, j * 128:(j + 1) * 128] for u in range(m // 4)), 0.0)
                ol[j] = _round(o * rl[j])

        def stage(g, *, q_next, scores, pv, wo):
            mxu, vpu, n_vpu = [], (), 0
            if scores:
                mxu.append((mxu_scores(g), NC * nt))
            if wo:
                mxu.append((mxu_wo(g - 2), NC * KC))
            if q_next:
                mxu.append((mxu_q(g + 1, 0), NC * KC))
            if pv:
                mxu.append((mxu_pv(*pv), NC * pv[0]))
                vpu, n_vpu = vpu_pv(g - 1, pv[0]), (nt - pv[0]) * PR // 16
            _interleave((w for s, _ in mxu for w in s), sum(n for _, n in mxu), vpu, n_vpu)
            if pv:
                pv_finish(pv[0])
            if scores:
                softmax()
            if q_next:
                q_finish(0)

        def run(stream):
            for _ in stream:
                pass

        def ffn(x, loading):
            xn, factor = _layernorm(x)
            if loading:
                wait(w13_copy)
            h = []
            for f in range(FC):
                gate, up = (
                    _round(factor * _tree_sum(
                        _mm(xn[:, c * 128:(c + 1) * 128], w[f, c * 64:(c + 1) * 64, :])
                        for c in range(KC)))
                    for w in (w1b, w3b))
                h.append(_round(_round(gate * jax.nn.sigmoid(gate)) * up))
            y = [None] * KC
            for c, size in enumerate(W2_CHUNKS):
                if loading:
                    wait(w2_copy(c))
                for f in range(sum(W2_CHUNKS[:c]), sum(W2_CHUNKS[:c + 1])):
                    for n in range(KC):
                        r = _mm(h[f], w2b[n, f * 64:(f + 1) * 64, :])
                        y[n] = r if y[n] is None else y[n] + r
            xs[...] = _round(x + _round(jnp.concatenate(y, axis=1)))

        def transpose(m, slot, t0):
            def one(i, carry):
                for j in range(NC):
                    at = (slot, t0 + i, slice(j * 64, (j + 1) * 64))
                    mb[at] = pltpu.bitcast(_bf(mb[at]).astype(F32).T.astype(BF16), U32)
                return carry
            lax.fori_loop(0, m, one, 0)

        def layer(it, carry):
            z = it >> 1

            def first_layer(await_, start_, *fresh):
                @pl.when(it == 0)
                def _():
                    start(start_)
                    wait(await_)
                    for tiles_ in fresh:
                        transpose(*tiles_)

            def pv(g):
                return M_STEADY, g, T_V

            def v_steady(g):
                return v_head(g, *pv(g), sem_v.at[g]) + v_rest(g, M_STEADY)

            pv_last = (M_LAST, NP + z, NC)
            pv_first = (M_FIRST, NP + z, NC + M_LAST)
            pv_penult = (M_PENULT, NP + z, NC + M_LAST + M_FIRST)
            v_last = v_rest(NP - 1, M_LAST)

            v_first, v_penult = v_rest(0, pv_first[0]), v_rest(NP - 2, pv_penult[0])
            v_spare = sum((v_head(g, *at, sem_w.at[4]) for g, at in
                           ((NP - 1, pv_last), (0, pv_first), (NP - 2, pv_penult))), [])

            first_layer(wo_copy + wq_copy + k_copy(0), v_spare + k_copy(1) + v_first)
            xn_s[...], xf[...] = _layernorm(xs[...])
            run(mxu_q(0, 0))
            run(mxu_q(1, 1))
            q_finish(0)
            stage(z, q_next=False, scores=True, pv=None, wo=False)
            run(mxu_q(2, 0))
            q_finish(1)
            first_layer(v_spare + k_copy(1) + v_first, k_copy(2) + v_steady(1),
                        (M_LAST + pv_first[0] + pv_penult[0], NP, NC))
            stage(1 + z, q_next=False, scores=True, pv=pv_first, wo=False)
            q_finish(0)

            def body(g, carry):
                @pl.when(it == 0)
                def _():
                    start(k_copy(g + 1))
                    pl.when(g < NP - 2)(lambda: start(v_steady(g)))
                    pl.when(g == NP - 2)(lambda: start(v_penult))
                    wait(k_copy(g) + v_steady(g - 1))
                    transpose(*pv(g - 1))
                stage(g, q_next=True, scores=True, pv=pv(g - 1), wo=True)
                return carry

            lax.fori_loop(2, NP - 1, body, 0)
            first_layer(k_copy(NP - 1) + v_penult, v_last)
            stage(NP - 1 + z, q_next=False, scores=True, pv=pv_penult, wo=True)
            first_layer(v_last, w13_copy + sum((w2_copy(c) for c in range(len(W2_CHUNKS))), []))
            y = yp[0, 0]
            for i in range(1, (NP - 2) * NC):
                y = y + yp[i // NC, i % NC]
            yp[0, 0] = y
            stage(NP + z, q_next=False, scores=False, pv=pv_last, wo=True)
            run(mxu_wo(NP - 1))
            y = _tree_sum(yp[g, j] for g, j in
                          [(0, 0)] + [(g, j) for g in (NP - 2, NP - 1) for j in range(NC)])
            xs[...] = _round(xs[...] + _round(jnp.sum(y, axis=0, keepdims=True)))
            pl.when(it == 0)(lambda: ffn(xs[...], True))
            pl.when(it != 0)(lambda: ffn(xs[...], False))
            return carry

        dg[...] = jnp.zeros_like(dg)
        x_copy.wait()
        xs[...] = jnp.broadcast_to(xb[0].astype(F32), (8, D))
        lax.fori_loop(0, 2, layer, 0)
        o_ref[0] = xs[0:1, :].astype(o_ref.dtype)

    return kernel, nu, n_slots


@jax.jit
def pallas_interleave_layers__sliding_block_cached__glu_gated_swiglu__decode_kernel(
    A_x: jax.Array,
    A_k_cache: jax.Array,
    A_v_cache: jax.Array,
    A_wq: jax.Array,
    A_wo: jax.Array,
    B_x: jax.Array,
    B_w1: jax.Array,
    B_w3: jax.Array,
    B_w2: jax.Array,
):
    del B_x
    sk = A_k_cache.shape[2]
    win = min(4096, max(256, sk // 4))
    assert A_x.shape == (1, 1, D) and A_k_cache.shape == (1, HQ, sk, DH)
    assert win == 4096 and sk % 128 == 0
    kernel, nu, n_slots = _make_kernel(sk - win, win)

    def as_rows(c):
        return jnp.swapaxes(c, 2, 3).reshape(NP, PR, sk)

    return pl.pallas_call(
        kernel,
        out_shape=jax.ShapeDtypeStruct((1, 1, D), A_x.dtype),
        in_specs=[pl.BlockSpec(memory_space=pl.ANY)] * 8,
        scratch_shapes=[
            pltpu.VMEM((NP + 1, n_slots, PR // 2, 128), U32),
            pltpu.VMEM((NP, 4 * nu - M_STEADY, PR // 2, 128), U32),
            pltpu.VMEM((FC, D // 2, 128), U32),
            pltpu.VMEM((FC, D // 2, 128), U32),
            pltpu.VMEM((KC, FF // 2, 128), U32),
            pltpu.VMEM((1, 1, D), BF16),
            pltpu.VMEM((8, D), F32),
            pltpu.VMEM((8, D), F32),
            pltpu.VMEM((8, 128), F32),
            pltpu.VMEM((2, KC, 8, PR), F32),
            pltpu.VMEM((NC, 8, 128), F32),
            pltpu.VMEM((nu, 8, 128), F32),
            pltpu.VMEM((nu, 8, 128), F32),
            pltpu.VMEM((nu, 8, 128), F32),
            pltpu.VMEM((2, 4 * nu, 8, 128), F32),
            pltpu.VMEM((NC, 8, 128), F32),
            pltpu.VMEM((NC, 8, 128), F32),
            pltpu.VMEM((nu, 8, PR), F32),
            pltpu.VMEM((NC, 8, 128), F32),
            pltpu.VMEM((NP, NC, 8, D), F32),
            pltpu.SemaphoreType.DMA((NP,)),
            pltpu.SemaphoreType.DMA((NP,)),
            pltpu.SemaphoreType.DMA((5 + len(W2_CHUNKS),)),
        ],
        compiler_params=pltpu.CompilerParams(
            vmem_limit_bytes=128 * 1024 * 1024, disable_semaphore_checks=True),
        name="interleave_decode",
    )(A_x, as_rows(A_k_cache), as_rows(A_v_cache), A_wq, A_wo.reshape(NP, PR, D),
      B_w1, B_w3, B_w2)
```

```python
import jax
import jax.numpy as jnp
from jax import lax
import jax.experimental.pallas as pl
import jax.experimental.pallas.tpu as pltpu

F32, BF16, U32 = jnp.float32, jnp.bfloat16, jnp.uint32

D, HQ, DH, FF = 640, 32, 192, 1536
NP = HQ // 2
PR = 2 * DH
KC, NC, FC = D // 128, PR // 128, FF // 128
EPS = 1e-5
SCALE = DH ** -0.5

M_STEADY = 4
M_FIRST = 8
M_PENULT = 8
M_LAST = 16
W2_CHUNKS = (8, 3, 1)
PV_BLOCK = 3
PACE_EVERY = 7


def _bf(w):
    return pltpu.bitcast(w, BF16)


def _mm(lhs, w):
    return lax.dot_general(lhs, _bf(w), (((1,), (0,)), ((), ())),
                           preferred_element_type=F32)


def _round(x):
    return x.astype(BF16).astype(F32)


def _tree_sum(xs):
    xs = list(xs)
    while len(xs) > 1:
        xs = [xs[i] + xs[i + 1] if i + 1 < len(xs) else xs[i]
              for i in range(0, len(xs), 2)]
    return xs[0]


def _layernorm(x):
    xs = [x[:, c * 128:(c + 1) * 128] for c in range(KC)]
    c = x - jnp.sum(_tree_sum(xs), axis=-1, keepdims=True) * (1.0 / D)
    sq = _tree_sum(c[:, i * 128:(i + 1) * 128] ** 2 for i in range(KC))
    v = jnp.sum(sq, axis=-1, keepdims=True) * (1.0 / D)
    return _round(c), jnp.broadcast_to(lax.rsqrt(v + EPS), (8, 128))


def _interleave(a, na, b, nb):
    ia = ib = 0
    for w in b:
        ib += w
        while ia * nb < ib * na:
            ia += next(a, na)
    for _ in a:
        pass


def _make_kernel(s0, win):
    nt = win // 128
    nu = nt // 4
    T_WO = nt
    T_WQ = T_WO + KC
    T_V = T_WQ + 2 * NC
    n_slots = max(T_V + M_STEADY, NC + M_LAST + M_FIRST + M_PENULT)

    def kernel(x_hbm, k_hbm, v_hbm, wq_hbm, wo_hbm, w1_hbm, w3_hbm, w2_hbm, o_ref,
               mb, vb, w1b, w3b, w2b, xb,
               xs, xn_s, xf, qp, ql, sa, sb, pb, pbb, rl, dg, ox, ol, yp,
               sem_k, sem_v, sem_w):
        row = lax.broadcasted_iota(jnp.int32, (8, 128), 0)
        lane = lax.broadcasted_iota(jnp.int32, (8, 128), 1)

        def group(n, src, buf, idx, sem):
            def copy(i):
                return pltpu.make_async_copy(src(i), buf.bitcast(BF16).at[idx(i)], sem)
            return n, copy

        def col(i, base=0):
            return pl.ds(pl.multiple_of(base + i * 128, 128), 128)

        def start(groups):
            for n, copy in groups:
                lax.fori_loop(0, n, lambda i, c: (copy(i).start(), c)[1], 0)

        def wait(groups):
            for n, copy in groups:
                lax.fori_loop(0, n, lambda i, c: (copy(i).wait(), c)[1], 0)

        def k_copy(g):
            return [group(nt, lambda i: k_hbm.at[g, :, col(i, s0)],
                          mb, lambda i: (g, i), sem_k.at[g & 1])]

        def v_head(g, m, slot, t0, sem):
            return [group(m, lambda i: v_hbm.at[g, :, col(i, s0)],
                          mb, lambda i: (slot, t0 + i), sem)]

        def v_rest(g, m):
            return [group(nt - m, lambda i: v_hbm.at[g, :, col(i, s0 + m * 128)],
                          vb, lambda i: (g, m - M_STEADY + i), sem_v.at[g & 1])]

        x_copy = pltpu.make_async_copy(x_hbm, xb, sem_w.at[0])

        def rows(r, n=128):
            return pl.ds(pl.multiple_of(r * n, n), n)

        def tiles(src, r0, n_rows, n_cols, buf, idx, sem):
            def at(i):
                return r0 + lax.div(i, n_cols), lax.rem(i, n_cols)
            return group(n_rows * n_cols, lambda i: src.at[rows(at(i)[0]), col(at(i)[1])],
                         buf, lambda i: idx(*at(i)), sem)

        wq_copy = [
            group(NP * NC, lambda i, c=c: wq_hbm.at[pl.ds(c * 128, 128), col(i)], mb,
                  lambda i, c=c: (lax.div(i, NC), T_WQ + 2 * lax.rem(i, NC) + c // NC,
                                  pl.ds(c % NC * 128, 128)),
                  sem_w.at[1])
            for c in range(KC)]
        wo_copy = [group(NP * KC,
                         lambda i: wo_hbm.at[lax.div(i, KC), :, col(lax.rem(i, KC))], mb,
                         lambda i: (lax.div(i, KC), T_WO + lax.rem(i, KC)), sem_w.at[1])]
        w13_copy = [tiles(w, 0, KC, FC, b, lambda r, c: (c, rows(r)), sem_w.at[0])
                    for w, b in ((w1_hbm, w1b), (w3_hbm, w3b))]

        def w2_copy(c):
            return [tiles(w2_hbm, sum(W2_CHUNKS[:c]), W2_CHUNKS[c], KC, w2b,
                          lambda r, c: (c, rows(r)), sem_w.at[1 + c])]

        start(wo_copy)
        x_copy.start()
        start(wq_copy + k_copy(0))

        def mxu_scores(g):
            lhs = [ql[j] for j in range(NC)]
            for t in range(nt):
                u, r = t // 4, 2 * (t % 4)
                sa[u, r:r + 1, :] = _mm(lhs[0], mb[g, t, 0:64, :])[r:r + 1]
                yield 1
                sb[u, r:r + 2, :] = _mm(lhs[1], mb[g, t, 64:128, :])[r:r + 2]
                yield 1
                sa[u, r + 1:r + 2, :] = _mm(lhs[2], mb[g, t, 128:192, :])[r + 1:r + 2]
                yield 1

        def mxu_q(g, slot):
            for n in range(NC):
                for c in range(KC):
                    r0 = c % NC * 64
                    qp[slot, c, :, n * 128:(n + 1) * 128] = _mm(
                        xn_s[:, c * 128:(c + 1) * 128],
                        mb[g, T_WQ + 2 * n + c // NC, r0:r0 + 64, :])
                    yield 1

        def mxu_wo(g):
            for j in range(NC):
                o = ol[j]
                for n in range(KC):
                    yp[g, j, :, n * 128:(n + 1) * 128] = _mm(
                        o, mb[g, T_WO + n, j * 64:(j + 1) * 64, :])
                    yield 1

        def mxu_pv(m, slot, t0):
            for t in range(m):
                u, r = t // 4, 2 * (t % 4)
                p = _round(pb[u])
                for j in range(NC):
                    ox[u, r:r + 2, j * 128:(j + 1) * 128] = _mm(
                        p, mb[slot, t0 + t, j * 64:(j + 1) * 64, :])[r:r + 2]
                    yield 1

        def vpu_pv(g, m):
            for h in range(2):
                for i0 in range(0, DH // 16, PV_BLOCK):
                    acc = [None] * PV_BLOCK
                    for t in range(m, nt):
                        if i0 == 0:
                            r = 2 * (t % 4) + h
                            p = jnp.broadcast_to(pb[t // 4, r:r + 1, :], (8, 128))
                            pbb[h, t] = p
                        else:
                            p = pbb[h, t]
                        p = jnp.concatenate([p, p], axis=0)
                        for i in range(PV_BLOCK):
                            r0 = h * (DH // 2) + (i0 + i) * 8
                            v = _bf(vb[g, t - M_STEADY, r0:r0 + 8, :]).astype(F32) * p
                            acc[i] = v if acc[i] is None else acc[i] + v
                        if (nt - 1 - t) % PACE_EVERY == 0:
                            for i in range(PV_BLOCK):
                                mb[NP, 0, i * 16:(i + 1) * 16, :] = pltpu.bitcast(acc[i], U32)
                        if t == nt - 1:
                            sums = [jnp.sum(x[k:k + 8], axis=1, keepdims=True)
                                    for x in acc for k in (0, 8)]
                            for i, x in enumerate(sums):
                                j, c0 = divmod(h * DH + i0 * 16 + i * 8, 128)
                                x = jnp.broadcast_to(x, (8, 128))
                                dg[j, :, c0:c0 + 8] = x[:, c0:c0 + 8]
                        yield PV_BLOCK

        def per_head(x, op):
            x = op(x, pltpu.roll(x, 2, 0))
            return op(x, pltpu.roll(x, 4, 0))

        def q_finish(slot):
            q = _tree_sum(qp[slot, c] for c in range(KC))
            q = _round(q * jnp.concatenate([xf[...]] * NC, axis=1))
            ql[0] = q[:, :128]
            ql[1] = jnp.where((row & 1) == (lane >> 6), q[:, 128:256], 0.0)
            ql[2] = q[:, 256:]

        def softmax():
            s = [sa[u] + sb[u] for u in range(nu)]
            m = s[0]
            for x in s[1:]:
                m = jnp.maximum(m, x)
            m = jnp.max(per_head(m, jnp.maximum), axis=1, keepdims=True)
            p = [jnp.exp((x - m) * SCALE) for x in s]
            l = jnp.sum(per_head(_tree_sum(p), jnp.add), axis=1, keepdims=True)
            inv = jnp.broadcast_to(1.0 / l, (8, 128))
            inv_o = pltpu.roll(inv, 1, 0)
            even = (row & 1) == 0
            inv_a, inv_b = jnp.where(even, inv, inv_o), jnp.where(even, inv_o, inv)
            for u in range(nu):
                pb[u] = p[u]
            rl[0], rl[1], rl[2] = inv_a, jnp.where(lane < 64, inv_a, inv_b), inv_b

        def pv_finish(m):
            own = ((row & 1) == 0, (row & 1) == (lane >> 6), (row & 1) == 1)
            for j in range(NC):
                o = jnp.where((lane & 7) == row, dg[j], 0.0) + jnp.where(own[j], _tree_sum(
                    ox[u, :, j * 128:(j + 1) * 128] for u in range(m // 4)), 0.0)
                ol[j] = _round(o * rl[j])

        def stage(g, *, q_next, scores, pv, wo):
            mxu, vpu, n_vpu = [], (), 0
            if scores:
                mxu.append((mxu_scores(g), NC * nt))
            if wo:
                mxu.append((mxu_wo(g - 2), NC * KC))
            if q_next:
                mxu.append((mxu_q(g + 1, 0), NC * KC))
            if pv:
                mxu.append((mxu_pv(*pv), NC * pv[0]))
                vpu, n_vpu = vpu_pv(g - 1, pv[0]), (nt - pv[0]) * PR // 16
            _interleave((w for s, _ in mxu for w in s), sum(n for _, n in mxu), vpu, n_vpu)
            if pv:
                pv_finish(pv[0])
            if scores:
                softmax()
            if q_next:
                q_finish(0)

        def run(stream):
            for _ in stream:
                pass

        def ffn(x, loading):
            xn, factor = _layernorm(x)
            if loading:
                wait(w13_copy)
            h = []
            for f in range(FC):
                gate, up = (
                    _round(factor * _tree_sum(
                        _mm(xn[:, c * 128:(c + 1) * 128], w[f, c * 64:(c + 1) * 64, :])
                        for c in range(KC)))
                    for w in (w1b, w3b))
                h.append(_round(_round(gate * jax.nn.sigmoid(gate)) * up))
            y = [None] * KC
            for c, size in enumerate(W2_CHUNKS):
                if loading:
                    wait(w2_copy(c))
                for f in range(sum(W2_CHUNKS[:c]), sum(W2_CHUNKS[:c + 1])):
                    for n in range(KC):
                        r = _mm(h[f], w2b[n, f * 64:(f + 1) * 64, :])
                        y[n] = r if y[n] is None else y[n] + r
            xs[...] = _round(x + _round(jnp.concatenate(y, axis=1)))

        def transpose(m, slot, t0):
            def one(i, carry):
                for j in range(NC):
                    at = (slot, t0 + i, slice(j * 64, (j + 1) * 64))
                    mb[at] = pltpu.bitcast(_bf(mb[at]).astype(F32).T.astype(BF16), U32)
                return carry
            lax.fori_loop(0, m, one, 0)

        def layer(it, carry):
            z = it >> 1

            def first_layer(await_, start_, *fresh):
                @pl.when(it == 0)
                def _():
                    start(start_)
                    wait(await_)
                    for tiles_ in fresh:
                        transpose(*tiles_)

            def pv(g):
                return M_STEADY, g, T_V

            def v_steady(g):
                return v_head(g, *pv(g), sem_v.at[g & 1]) + v_rest(g, M_STEADY)

            pv_last = (M_LAST, NP + z, NC)
            pv_first = (M_FIRST, NP + z, NC + M_LAST)
            pv_penult = (M_PENULT, NP + z, NC + M_LAST + M_FIRST)
            v_last = v_rest(NP - 1, M_LAST)

            v_first, v_penult = v_rest(0, pv_first[0]), v_rest(NP - 2, pv_penult[0])
            v_spare = sum((v_head(g, *at, sem_w.at[2]) for g, at in
                           ((NP - 1, pv_last), (0, pv_first), (NP - 2, pv_penult))), [])

            first_layer(wo_copy + wq_copy + k_copy(0), v_spare + k_copy(1) + v_first)
            xn_s[...], xf[...] = _layernorm(xs[...])
            run(mxu_q(0, 0))
            run(mxu_q(1, 1))
            q_finish(0)
            stage(z, q_next=False, scores=True, pv=None, wo=False)
            run(mxu_q(2, 0))
            q_finish(1)
            first_layer(v_spare + k_copy(1) + v_first, k_copy(2) + v_steady(1),
                        (M_LAST + pv_first[0] + pv_penult[0], NP, NC))
            stage(1 + z, q_next=False, scores=True, pv=pv_first, wo=False)
            q_finish(0)

            def body(g, carry):
                @pl.when(it == 0)
                def _():
                    start(k_copy(g + 1))
                    pl.when(g < NP - 2)(lambda: start(v_steady(g)))
                    pl.when(g == NP - 2)(lambda: start(v_penult))
                    wait(k_copy(g) + v_steady(g - 1))
                    transpose(*pv(g - 1))
                stage(g, q_next=True, scores=True, pv=pv(g - 1), wo=True)
                return carry

            lax.fori_loop(2, NP - 1, body, 0)
            first_layer(k_copy(NP - 1) + v_penult, v_last)
            stage(NP - 1 + z, q_next=False, scores=True, pv=pv_penult, wo=True)
            first_layer(v_last, w13_copy + sum((w2_copy(c) for c in range(len(W2_CHUNKS))), []))
            y = yp[0, 0]
            for i in range(1, (NP - 2) * NC):
                y = y + yp[i // NC, i % NC]
            yp[0, 0] = y
            stage(NP + z, q_next=False, scores=False, pv=pv_last, wo=True)
            run(mxu_wo(NP - 1))
            y = _tree_sum(yp[g, j] for g, j in
                          [(0, 0)] + [(g, j) for g in (NP - 2, NP - 1) for j in range(NC)])
            xs[...] = _round(xs[...] + _round(jnp.sum(y, axis=0, keepdims=True)))
            pl.when(it == 0)(lambda: ffn(xs[...], True))
            pl.when(it != 0)(lambda: ffn(xs[...], False))
            return carry

        dg[...] = jnp.zeros_like(dg)
        x_copy.wait()
        xs[...] = jnp.broadcast_to(xb[0].astype(F32), (8, D))
        lax.fori_loop(0, 2, layer, 0)
        o_ref[0] = xs[0:1, :].astype(o_ref.dtype)

    return kernel, nu, n_slots


@jax.jit
def pallas_interleave_layers__sliding_block_cached__glu_gated_swiglu__decode_kernel(
    A_x: jax.Array,
    A_k_cache: jax.Array,
    A_v_cache: jax.Array,
    A_wq: jax.Array,
    A_wo: jax.Array,
    B_x: jax.Array,
    B_w1: jax.Array,
    B_w3: jax.Array,
    B_w2: jax.Array,
):
    del B_x
    sk = A_k_cache.shape[2]
    win = min(4096, max(256, sk // 4))
    assert A_x.shape == (1, 1, D) and A_k_cache.shape == (1, HQ, sk, DH)
    assert win == 4096 and sk % 128 == 0
    kernel, nu, n_slots = _make_kernel(sk - win, win)

    def as_rows(c):
        return jnp.swapaxes(c, 2, 3).reshape(NP, PR, sk)

    return pl.pallas_call(
        kernel,
        out_shape=jax.ShapeDtypeStruct((1, 1, D), A_x.dtype),
        in_specs=[pl.BlockSpec(memory_space=pl.ANY)] * 8,
        scratch_shapes=[
            pltpu.VMEM((NP + 1, n_slots, PR // 2, 128), U32),
            pltpu.VMEM((NP, 4 * nu - M_STEADY, PR // 2, 128), U32),
            pltpu.VMEM((FC, D // 2, 128), U32),
            pltpu.VMEM((FC, D // 2, 128), U32),
            pltpu.VMEM((KC, FF // 2, 128), U32),
            pltpu.VMEM((1, 1, D), BF16),
            pltpu.VMEM((8, D), F32),
            pltpu.VMEM((8, D), F32),
            pltpu.VMEM((8, 128), F32),
            pltpu.VMEM((2, KC, 8, PR), F32),
            pltpu.VMEM((NC, 8, 128), F32),
            pltpu.VMEM((nu, 8, 128), F32),
            pltpu.VMEM((nu, 8, 128), F32),
            pltpu.VMEM((nu, 8, 128), F32),
            pltpu.VMEM((2, 4 * nu, 8, 128), F32),
            pltpu.VMEM((NC, 8, 128), F32),
            pltpu.VMEM((NC, 8, 128), F32),
            pltpu.VMEM((nu, 8, PR), F32),
            pltpu.VMEM((NC, 8, 128), F32),
            pltpu.VMEM((NP, NC, 8, D), F32),
            pltpu.SemaphoreType.DMA((2,)),
            pltpu.SemaphoreType.DMA((2,)),
            pltpu.SemaphoreType.DMA((1 + len(W2_CHUNKS),)),
        ],
        compiler_params=pltpu.CompilerParams(vmem_limit_bytes=128 * 1024 * 1024),
        name="interleave_decode",
    )(A_x, as_rows(A_k_cache), as_rows(A_v_cache), A_wq, A_wo.reshape(NP, PR, D),
      B_w1, B_w3, B_w2)
```
